```python
import jax
import jax.numpy as jnp

def _softmax(x, axis=-1):
    return jax.nn.softmax(x, axis=axis)
def _gelu(x):
    return jax.nn.gelu(x, approximate=True)
def _silu(x):
    return jax.nn.silu(x)
def _sigmoid(x):
    return jax.nn.sigmoid(x)
def _layernorm(x, axis=-1, eps=1e-5):
    m = jnp.mean(x, axis=axis, keepdims=True)
    v = jnp.var(x, axis=axis, keepdims=True)
    return (x - m) / jnp.sqrt(v + eps)
def _scatter_add(tgt, idx, src, axis=0):
    return tgt.at[idx].add(src)
def _segment_sum(src, seg, n):
    return jax.ops.segment_sum(src, seg, n)
class _Rng:
    def __init__(self, key):
        self._k = key
    def _next(self):
        self._k, sub = jax.random.split(self._k)
        return sub
    def normal(self, shape):
        return jax.random.normal(self._next(), shape, dtype=jnp.bfloat16)
    def randint(self, lo, hi, shape):
        return jax.random.randint(self._next(), shape, lo, hi, dtype=jnp.int32)
    def uniform(self, shape, lo=0.0, hi=1.0):
        return jax.random.uniform(self._next(), shape, jnp.bfloat16, lo, hi)
    def permutation(self, n):
        return jax.random.permutation(self._next(), n)


kernel_name = 'recurrent_scan__compressed_kv_cla__dense_activation_silu__decode'

def setup_inputs():
    _rng = _Rng(jax.random.key(int.from_bytes(__import__("os").urandom(4), "little")))
    _w = (lambda a: (lambda t: t.astype(jnp.bfloat16) if jnp.issubdtype(t.dtype, jnp.floating) else t)(jnp.asarray(a)))
    def _A_setup():
        B, H, Sq, Sk, D, M = 1, 32, 1, 32768, 128, 512
        Dc = 4 * D
        return {
            "x": _w((lambda *s: _rng.normal(s) * 0.05)(B, Sq, M)),
            "c_kv": _w((lambda *s: _rng.normal(s) * 0.05)(B, Sk, Dc)),
            "w_q": _w((lambda *s: _rng.normal(s) * 0.05)(M, H, D) * (M ** -0.5)),
            "w_uk": _w((lambda *s: _rng.normal(s) * 0.05)(Dc, H, D) * (Dc ** -0.5)),
            "w_uv": _w((lambda *s: _rng.normal(s) * 0.05)(Dc, H, D) * (Dc ** -0.5)),
            "w_o": _w((lambda *s: _rng.normal(s) * 0.05)(H, D, M) * ((H * D) ** -0.5)),
        }
    _A_in = _A_setup()

    def _B_setup():
        B, S, D, F = 1, 1, 512, 1376
        return {
            "x": _w((lambda *s: _rng.normal(s) * 0.05)(B, S, D)),
            "w1": _w((lambda *s: _rng.normal(s) * 0.05)(D, F) * (D ** -0.5)),
            "w2": _w((lambda *s: _rng.normal(s) * 0.05)(F, D) * (F ** -0.5)),
        }
    _B_in = _B_setup()

    return {
        "A_x": _A_in["x"],
        "A_c_kv": _A_in["c_kv"],
        "A_w_q": _A_in["w_q"],
        "A_w_uk": _A_in["w_uk"],
        "A_w_uv": _A_in["w_uv"],
        "A_w_o": _A_in["w_o"],
        "B_x": _B_in["x"],
        "B_w1": _B_in["w1"],
        "B_w2": _B_in["w2"],
    }

def reference(A_x, A_c_kv, A_w_q, A_w_uk, A_w_uv, A_w_o, B_x, B_w1, B_w2):
    def _A_ref(x, c_kv, w_q, w_uk, w_uv, w_o):
        B, Sq, M = x.shape[0], x.shape[1], x.shape[2]
        Sk = c_kv.shape[1]
        H, D = w_q.shape[1], w_q.shape[2]
        q = jnp.einsum("bqm,mhd->bhqd", x, w_q)
        k = jnp.einsum("bkc,chd->bhkd", c_kv, w_uk)
        v = jnp.einsum("bkc,chd->bhkd", c_kv, w_uv)
        scores = jnp.einsum("bhqd,bhkd->bhqk", q, k) * (D ** -0.5)
        off = Sk - Sq
        qi = jnp.arange(Sq)[:, None]
        kj = jnp.arange(Sk)[None, :]
        cmask = kj <= (qi + off)
        scores = jnp.where(cmask[None, None], scores, -1e9)
        p = _softmax(scores, axis=-1)
        ctx = jnp.einsum("bhqk,bhkd->bhqd", p, v)
        return jnp.einsum("bhqd,hdm->bqm", ctx, w_o)

    def _B_ref(x, w1, w2):
        h = jnp.einsum("bsd,df->bsf", x, w1)
        h = _silu(h)
        out = jnp.einsum("bsf,fd->bsd", h, w2)
        return out

    x = A_x
    xn = _layernorm(x, axis=-1)
    s = _A_ref(xn, A_c_kv, A_w_q, A_w_uk, A_w_uv, A_w_o)
    g = _silu(_B_ref(xn, B_w1, B_w2))
    return x + s * g
```

```python
import functools

import jax
import jax.numpy as jnp
from jax import lax
import jax.experimental.pallas as pl
import jax.experimental.pallas.tpu as pltpu

_F32 = jnp.float32
_BF16 = jnp.bfloat16
_NT = (((1,), (1,)), ((), ()))


def _silu(v):
    return v / (1.0 + jnp.exp(-v))


def _kernel(x_hbm, ckv_hbm, wq_hbm, wuk_hbm, wuv_hbm, wo_hbm, w1_hbm, w2_hbm,
            o_ref,
            x_v, ckv_v, wq_v, wuk_v, wuv_v, wo_v, w1_v, w2_v, e_v,
            sems,
            *, H, D, M, C, SK, TK, NW, eps):
    nck = SK // TK
    HC = H * C
    WCH = HC // NW
    G = 128 * H

    sem_x, sem_f = 0, 1
    sem_q, sem_k, sem_v, sem_o = 3, 3 + NW, 3 + 2 * NW, 3 + 3 * NW
    sem_c = 3 + 4 * NW

    def chunk_copy(src, dst, sem, i, rows):
        return pltpu.make_async_copy(src.at[pl.ds(i * rows, rows)],
                                     dst.at[pl.ds(i * rows, rows)], sems.at[sem + i])

    x_cp = pltpu.make_async_copy(x_hbm, x_v, sems.at[sem_x])
    wq_cp = [chunk_copy(wq_hbm, wq_v, sem_q, i, WCH) for i in range(NW)]
    wuk_cp = [chunk_copy(wuk_hbm, wuk_v, sem_k, i, WCH) for i in range(NW)]
    wuv_cp = [chunk_copy(wuv_hbm, wuv_v, sem_v, i, WCH) for i in range(NW)]
    OCH = (H * D) // NW
    wo_cp = [chunk_copy(wo_hbm, wo_v, sem_o, i, OCH) for i in range(NW)]
    w1_cp = pltpu.make_async_copy(w1_hbm, w1_v, sems.at[sem_f])
    w2_cp = pltpu.make_async_copy(w2_hbm, w2_v, sems.at[sem_f + 1])

    x_cp.start()
    for cp in wq_cp:
        cp.start()
    for cp in wuk_cp:
        cp.start()
    for i in range(nck):
        chunk_copy(ckv_hbm, ckv_v, sem_c, i, TK).start()
    w1_cp.start()
    w2_cp.start()
    for cp in wuv_cp:
        cp.start()
    for cp in wo_cp:
        cp.start()

    ei = lax.broadcasted_iota(jnp.int32, (128, G), 0)
    ej = lax.broadcasted_iota(jnp.int32, (128, G), 1)
    e_v[...] = jnp.where(ej // H == ei, 1.0, 0.0).astype(_BF16)
    di = lax.broadcasted_iota(jnp.int32, (H, G), 0)
    dj = lax.broadcasted_iota(jnp.int32, (H, G), 1)
    diag = (dj % H) == di

    def expand(rows_bf16):
        ex = jnp.dot(rows_bf16, e_v[...], preferred_element_type=_F32)
        return jnp.where(diag, ex, 0.0).astype(_BF16)

    x_cp.wait()
    x = x_v[...].astype(_F32)
    mu = jnp.mean(x, axis=-1, keepdims=True)
    xc = x - mu
    var = jnp.mean(xc * xc, axis=-1, keepdims=True)
    xn = (xc / jnp.sqrt(var + eps)).astype(_BF16)
    xn_h = jnp.broadcast_to(xn, (H, M))

    nblk = M // 128
    aq = [expand(xn_h[:, a * 128:(a + 1) * 128]) for a in range(nblk)]
    q = jnp.zeros((H, D), _F32)
    per = G // WCH if G >= WCH else 1
    for a in range(nblk):
        for i in range(NW):
            if i * WCH < (a + 1) * G and (i + 1) * WCH > a * G and i * WCH >= a * G:
                wq_cp[i].wait()
        q = q + jnp.dot(aq[a], wq_v[a * G:(a + 1) * G, :], preferred_element_type=_F32)
    q = q.astype(_BF16)

    scale = D ** -0.5
    ql = []
    for a in range(C // 128):
        for i in range(NW):
            if i * WCH >= a * G and i * WCH < (a + 1) * G:
                wuk_cp[i].wait()
        t = lax.dot_general(q, wuk_v[a * G:(a + 1) * G, :], _NT, preferred_element_type=_F32)
        t = jnp.where(diag, t * scale, 0.0).astype(_BF16)
        ql.append(lax.dot_general(t, e_v[...], _NT, preferred_element_type=_F32))
    q_lat = jnp.concatenate(ql, axis=-1).astype(_BF16)

    def body(i, carry):
        m_old, l_old, acc = carry
        chunk_copy(ckv_hbm, ckv_v, sem_c, i, TK).wait()
        kv = ckv_v[pl.ds(pl.multiple_of(i * TK, TK), TK), :]
        s = lax.dot_general(q_lat, kv, _NT, preferred_element_type=_F32)
        m_new = jnp.maximum(m_old, jnp.max(s, axis=-1, keepdims=True))
        alpha = jnp.exp(m_old - m_new)
        p = jnp.exp(s - m_new)
        l_new = alpha * l_old + jnp.sum(p, axis=-1, keepdims=True)
        acc = alpha * acc + jnp.dot(p.astype(_BF16), kv, preferred_element_type=_F32)
        return m_new, l_new, acc

    m0 = jnp.full((H, 1), -jnp.inf, _F32)
    l0 = jnp.zeros((H, 1), _F32)
    acc0 = jnp.zeros((H, C), _F32)
    _, l_fin, acc = lax.fori_loop(0, nck, body, (m0, l0, acc0))
    ctx_lat = (acc / l_fin).astype(_BF16)

    xn8 = jnp.broadcast_to(xn, (8, M))
    w1_cp.wait()
    h1 = lax.dot_general(xn8, w1_v[...], _NT, preferred_element_type=_F32)
    h1 = _silu(h1).astype(_BF16)
    w2_cp.wait()
    g = _silu(jnp.dot(h1, w2_v[...], preferred_element_type=_F32))[0:1]

    av = [expand(ctx_lat[:, a * 128:(a + 1) * 128]) for a in range(C // 128)]
    ctx = jnp.zeros((H, D), _F32)
    for a in range(C // 128):
        for i in range(NW):
            if i * WCH >= a * G and i * WCH < (a + 1) * G:
                wuv_cp[i].wait()
        ctx = ctx + jnp.dot(av[a], wuv_v[a * G:(a + 1) * G, :], preferred_element_type=_F32)

    hpc = H // NW
    ri = lax.broadcasted_iota(jnp.int32, (hpc, OCH), 0)
    rj = lax.broadcasted_iota(jnp.int32, (hpc, OCH), 1)
    bd = (rj // D) == ri
    so = jnp.zeros((hpc, M), _F32)
    for i in range(NW):
        cg = ctx[i * hpc:(i + 1) * hpc, :]
        lhs = jnp.where(bd, jnp.concatenate([cg] * hpc, axis=-1), 0.0).astype(_BF16)
        wo_cp[i].wait()
        so = so + jnp.dot(lhs, wo_v[i * OCH:(i + 1) * OCH, :], preferred_element_type=_F32)
    s = jnp.sum(so, axis=0, keepdims=True)

    o_ref[...] = (x + s * g).astype(o_ref.dtype)


@jax.jit
def pallas_recurrent_scan__compressed_kv_cla__dense_activation_silu__decode_kernel(
    A_x: jax.Array,
    A_c_kv: jax.Array,
    A_w_q: jax.Array,
    A_w_uk: jax.Array,
    A_w_uv: jax.Array,
    A_w_o: jax.Array,
    B_x: jax.Array,
    B_w1: jax.Array,
    B_w2: jax.Array,
):
    B, SQ, M = A_x.shape
    _, SK, C = A_c_kv.shape
    _, H, D = A_w_q.shape
    F = B_w1.shape[1]
    assert B == 1 and SQ == 1 and D == 128 and M % 128 == 0 and C % 128 == 0
    TK = 2048
    NW = 4
    dt = A_x.dtype

    kernel = functools.partial(_kernel, H=H, D=D, M=M, C=C, SK=SK, TK=TK, NW=NW, eps=1e-5)
    any_spec = pl.BlockSpec(memory_space=pl.ANY)
    out = pl.pallas_call(
        kernel,
        in_specs=[any_spec] * 8,
        out_specs=pl.BlockSpec(memory_space=pltpu.VMEM),
        out_shape=jax.ShapeDtypeStruct((1, M), dt),
        scratch_shapes=[
            pltpu.VMEM((1, M), dt),
            pltpu.VMEM((SK, C), dt),
            pltpu.VMEM((M * H, D), dt),
            pltpu.VMEM((C * H, D), dt),
            pltpu.VMEM((C * H, D), dt),
            pltpu.VMEM((H * D, M), dt),
            pltpu.VMEM((F, M), dt),
            pltpu.VMEM((F, M), dt),
            pltpu.VMEM((128, 128 * H), _BF16),
            pltpu.SemaphoreType.DMA((3 + 4 * NW + SK // TK,)),
        ],
        compiler_params=pltpu.CompilerParams(vmem_limit_bytes=100 * 1024 * 1024),
    )(
        A_x.reshape(1, M),
        A_c_kv.reshape(SK, C),
        A_w_q.reshape(M * H, D),
        A_w_uk.reshape(C * H, D),
        A_w_uv.reshape(C * H, D),
        A_w_o.reshape(H * D, M),
        B_w1.T,
        B_w2,
    )
    return out.reshape(B, SQ, M)
```

```python
import functools

import jax
import jax.numpy as jnp
from jax import lax
import jax.experimental.pallas as pl
import jax.experimental.pallas.tpu as pltpu

_F32 = jnp.float32
_BF16 = jnp.bfloat16
_NT = (((1,), (1,)), ((), ()))


def _silu(v):
    return v / (1.0 + jnp.exp(-v))


def _body(x_hbm, ckv_hbm, wq_hbm, wuk_hbm, wuv_hbm, wo_hbm, w1_hbm, w2_hbm,
          o_ref,
          x_v, ckv_v, wq_v, wuk_v, wuv_v, wo_v, w1_v, w2_v, e_v, sems,
          *, H, D, M, C, SK, TK, wo_mxu_heads, wo_vpu_rows, eps):
    nck = SK // TK
    G = 128 * H
    nq = M // 128
    nc = C // 128

    n_sem = [0]

    def copy(src, dst, lo=None, rows=None):
        sem = sems.at[n_sem[0]]
        n_sem[0] += 1
        if lo is None:
            return pltpu.make_async_copy(src, dst, sem)
        return pltpu.make_async_copy(src.at[pl.ds(lo, rows)], dst.at[pl.ds(lo, rows)], sem)

    def ckv_copy(i):
        return pltpu.make_async_copy(ckv_hbm.at[pl.ds(i * TK, TK)],
                                     ckv_v.at[pl.ds(i * TK, TK)], sems.at[i])

    n_sem[0] = nck
    x_cp = copy(x_hbm, x_v)
    wq_cp = [copy(wq_hbm, wq_v, a * G, G) for a in range(nq)]
    wuk_cp = [copy(wuk_hbm, wuk_v, a * G, G) for a in range(nc)]
    w1_cp = copy(w1_hbm, w1_v)
    w2_cp = copy(w2_hbm, w2_v)
    wuv_cp = [copy(wuv_hbm, wuv_v, a * G, G) for a in range(nc)]
    wo_cp = []
    lo = 0
    for nh in wo_mxu_heads:
        wo_cp.append(copy(wo_hbm, wo_v, lo, nh * D))
        lo += nh * D
    wo_tail_cp = []
    for rows in wo_vpu_rows:
        wo_tail_cp.append(copy(wo_hbm, wo_v, lo, rows))
        lo += rows
    assert lo == H * D and sum(wo_vpu_rows) == D

    x_cp.start()
    for cp in wq_cp + wuk_cp:
        cp.start()
    for i in range(nck):
        ckv_copy(i).start()
    for cp in [w1_cp, w2_cp] + wuv_cp + wo_cp + wo_tail_cp:
        cp.start()

    ei = lax.broadcasted_iota(jnp.int32, (128, G), 0)
    ej = lax.broadcasted_iota(jnp.int32, (128, G), 1)
    e_v[...] = jnp.where(ej // H == ei, 1.0, 0.0).astype(_BF16)
    di = lax.broadcasted_iota(jnp.int32, (H, G), 0)
    dj = lax.broadcasted_iota(jnp.int32, (H, G), 1)
    diag = (dj % H) == di

    def expand(rows_bf16):
        ex = jnp.dot(rows_bf16, e_v[...], preferred_element_type=_F32)
        return jnp.where(diag, ex, 0.0).astype(_BF16)

    x_cp.wait()
    x = x_v[...].astype(_F32)
    mu = jnp.mean(x, axis=-1, keepdims=True)
    xc = x - mu
    var = jnp.mean(xc * xc, axis=-1, keepdims=True)
    xn = (xc / jnp.sqrt(var + eps)).astype(_BF16)
    xn_h = jnp.broadcast_to(xn, (H, M))

    aq = [expand(xn_h[:, a * 128:(a + 1) * 128]) for a in range(nq)]
    q = jnp.zeros((H, D), _F32)
    for a in range(nq):
        wq_cp[a].wait()
        q = q + jnp.dot(aq[a], wq_v[a * G:(a + 1) * G, :], preferred_element_type=_F32)
    q = q.astype(_BF16)

    scale = D ** -0.5
    ql = []
    for a in range(nc):
        wuk_cp[a].wait()
        t = lax.dot_general(q, wuk_v[a * G:(a + 1) * G, :], _NT, preferred_element_type=_F32)
        t = jnp.where(diag, t * scale, 0.0).astype(_BF16)
        ql.append(lax.dot_general(t, e_v[...], _NT, preferred_element_type=_F32))
    q_lat = jnp.concatenate(ql, axis=-1).astype(_BF16)

    def step(i, carry):
        m_old, l_old, acc = carry
        ckv_copy(i).wait()
        kv = ckv_v[pl.ds(pl.multiple_of(i * TK, TK), TK), :]
        s = lax.dot_general(q_lat, kv, _NT, preferred_element_type=_F32)
        m_new = jnp.maximum(m_old, jnp.max(s, axis=-1, keepdims=True))
        alpha = jnp.exp(m_old - m_new)
        p = jnp.exp(s - m_new)
        l_new = alpha * l_old + jnp.sum(p, axis=-1, keepdims=True)
        acc = alpha * acc + jnp.dot(p.astype(_BF16), kv, preferred_element_type=_F32)
        return m_new, l_new, acc

    m0 = jnp.full((H, 1), -jnp.inf, _F32)
    l0 = jnp.zeros((H, 1), _F32)
    acc0 = jnp.zeros((H, C), _F32)
    _, l_fin, acc = lax.fori_loop(0, nck, step, (m0, l0, acc0))
    ctx_lat = (acc / l_fin).astype(_BF16)

    xn8 = jnp.broadcast_to(xn, (8, M))
    w1_cp.wait()
    h1 = lax.dot_general(xn8, w1_v[...], _NT, preferred_element_type=_F32)
    h1 = _silu(h1).astype(_BF16)
    w2_cp.wait()
    g = _silu(jnp.dot(h1, w2_v[...], preferred_element_type=_F32))[0:1]

    av = [expand(ctx_lat[:, a * 128:(a + 1) * 128]) for a in range(nc)]
    ctx = jnp.zeros((H, D), _F32)
    for a in range(nc):
        wuv_cp[a].wait()
        ctx = ctx + jnp.dot(av[a], wuv_v[a * G:(a + 1) * G, :], preferred_element_type=_F32)
    ctx = ctx.astype(_BF16).astype(_F32)

    row8 = lax.broadcasted_iota(jnp.int32, (8, D), 0)

    def head_lhs(h):
        grp = ctx[(h // 8) * 8:(h // 8) * 8 + 8, :]
        return jnp.where(row8 == (h % 8), grp, 0.0).astype(_BF16)

    eye = (lax.broadcasted_iota(jnp.int32, (D, D), 0)
           == lax.broadcasted_iota(jnp.int32, (D, D), 1))
    last = jnp.where(eye, jnp.broadcast_to(ctx[H - 1:H, :], (D, D)), 0.0).astype(_BF16)
    last_col = jnp.dot(last, jnp.ones((D, 128), _BF16), preferred_element_type=_F32)

    so8 = jnp.zeros((8, M), _F32)
    h0 = 0
    for cp, nh in zip(wo_cp, wo_mxu_heads):
        lhs = jnp.concatenate([head_lhs(h) for h in range(h0, h0 + nh)], axis=-1)
        cp.wait()
        so8 = so8 + jnp.dot(lhs, wo_v[h0 * D:(h0 + nh) * D, :], preferred_element_type=_F32)
        h0 += nh
    r0 = 0
    for cp, rows in zip(wo_tail_cp, wo_vpu_rows):
        coef = jnp.concatenate([last_col[r0:r0 + rows, :]] * (M // 128), axis=-1)
        cp.wait()
        w = wo_v[h0 * D + r0:h0 * D + r0 + rows, :].astype(_F32)
        prod = coef * w
        for r in range(0, rows, 8):
            so8 = so8 + prod[r:r + 8, :]
        r0 += rows
    s = jnp.sum(so8, axis=0, keepdims=True)

    o_ref[...] = (x + s * g).astype(o_ref.dtype)


def _kernel(*refs, n_sems, **kw):
    pl.run_scoped(lambda sems: _body(*refs, sems, **kw),
                  pltpu.SemaphoreType.DMA((n_sems,)))


@jax.jit
def pallas_recurrent_scan__compressed_kv_cla__dense_activation_silu__decode_kernel(
    A_x: jax.Array,
    A_c_kv: jax.Array,
    A_w_q: jax.Array,
    A_w_uk: jax.Array,
    A_w_uv: jax.Array,
    A_w_o: jax.Array,
    B_x: jax.Array,
    B_w1: jax.Array,
    B_w2: jax.Array,
):
    B, SQ, M = A_x.shape
    _, SK, C = A_c_kv.shape
    _, H, D = A_w_q.shape
    F = B_w1.shape[1]
    assert B == 1 and SQ == 1 and D == 128 and H == 32 and M % 128 == 0 and C % 128 == 0
    TK = 2048
    wo_mxu_heads = (8, 8, 8, 4, 2, 1)
    wo_vpu_rows = (96, 32)
    n_sems = SK // TK + 3 + M // 128 + 2 * (C // 128) + len(wo_mxu_heads) + len(wo_vpu_rows)
    dt = A_x.dtype

    kernel = functools.partial(
        _kernel, n_sems=n_sems, H=H, D=D, M=M, C=C, SK=SK, TK=TK,
        wo_mxu_heads=wo_mxu_heads, wo_vpu_rows=wo_vpu_rows, eps=1e-5)
    any_spec = pl.BlockSpec(memory_space=pl.ANY)
    out = pl.pallas_call(
        kernel,
        in_specs=[any_spec] * 8,
        out_specs=pl.BlockSpec(memory_space=pltpu.VMEM),
        out_shape=jax.ShapeDtypeStruct((1, M), dt),
        scratch_shapes=[
            pltpu.VMEM((1, M), dt),
            pltpu.VMEM((SK, C), dt),
            pltpu.VMEM((M * H, D), dt),
            pltpu.VMEM((C * H, D), dt),
            pltpu.VMEM((C * H, D), dt),
            pltpu.VMEM((H * D, M), dt),
            pltpu.VMEM((F, M), dt),
            pltpu.VMEM((F, M), dt),
            pltpu.VMEM((128, 128 * H), _BF16),
        ],
        compiler_params=pltpu.CompilerParams(vmem_limit_bytes=100 * 1024 * 1024),
    )(
        A_x.reshape(1, M),
        A_c_kv.reshape(SK, C),
        A_w_q.reshape(M * H, D),
        A_w_uk.reshape(C * H, D),
        A_w_uv.reshape(C * H, D),
        A_w_o.reshape(H * D, M),
        B_w1.T,
        B_w2,
    )
    return out.reshape(B, SQ, M)
```

```python
import functools

import jax
import jax.numpy as jnp
from jax import lax
import jax.experimental.pallas as pl
import jax.experimental.pallas.tpu as pltpu

_F32 = jnp.float32
_BF16 = jnp.bfloat16
_NT = (((1,), (1,)), ((), ()))


def _silu(v):
    return v / (1.0 + jnp.exp(-v))


def _body(x_hbm, ckv_hbm, wq_hbm, wuk_hbm, wuv_hbm, wo_hbm, w1_hbm, w2_hbm,
          o_ref,
          x_v, ckv_v, wq_v, wuk_v, wuv_v, wo_v, w1_v, w2_v, e_v, stage, sems,
          *, H, D, M, C, SK, TK, wo_mxu_heads, wo_vpu_rows, pre_hooks, post_hooks, eps):
    nck = SK // TK
    G = 128 * H
    nq = M // 128
    nc = C // 128
    F = w2_v.shape[0]

    n_sem = [0]

    def copy(src, dst, lo=None, rows=None):
        sem = sems.at[n_sem[0]]
        n_sem[0] += 1
        if lo is None:
            return pltpu.make_async_copy(src, dst, sem)
        return pltpu.make_async_copy(src.at[pl.ds(lo, rows)], dst.at[pl.ds(lo, rows)], sem)

    def ckv_copy(i):
        return pltpu.make_async_copy(ckv_hbm.at[pl.ds(i * TK, TK)],
                                     ckv_v.at[pl.ds(i * TK, TK)], sems.at[i])

    S, R, _ = stage.shape
    J0 = len(pre_hooks)
    NS = J0 + nck + len(post_hooks) - 2
    assert S == 3 and J0 >= 2 and len(post_hooks) >= 2 and NS * R <= F
    sem_h2s, sem_s2v = nck, nck + S

    def piece(j):
        return j * R if isinstance(j, int) else pl.multiple_of(j * R, 16)

    def h2s(j):
        return pltpu.make_async_copy(w2_hbm.at[pl.ds(piece(j), R)], stage.at[j % S],
                                     sems.at[sem_h2s + j % S])

    def s2v(j):
        return pltpu.make_async_copy(stage.at[j % S], w2_v.at[pl.ds(piece(j), R)],
                                     sems.at[sem_s2v + j % S])

    def side(j):
        static = isinstance(j, int)
        if not static or j < NS:
            h2s(j).start()
        if not static or 1 <= j <= NS:
            h2s(j - 1).wait()
            s2v(j - 1).start()
        if not static or 2 <= j <= NS + 1:
            s2v(j - 2).wait()

    def hook(name):
        if name in pre_hooks:
            side(pre_hooks.index(name))
        if name in post_hooks:
            side(J0 + nck + post_hooks.index(name))

    n_sem[0] = nck + 2 * S
    x_cp = copy(x_hbm, x_v)
    wq_cp = [copy(wq_hbm, wq_v, a * G, G) for a in range(nq)]
    wuk_cp = [copy(wuk_hbm, wuk_v, a * G, G) for a in range(nc)]
    ffn_cp = [copy(w1_hbm, w1_v)]
    if NS * R < F:
        ffn_cp.append(copy(w2_hbm, w2_v, NS * R, F - NS * R))
    wuv_cp = [copy(wuv_hbm, wuv_v, a * G, G) for a in range(nc)]
    wo_cp = []
    lo = 0
    for nh in wo_mxu_heads:
        wo_cp.append(copy(wo_hbm, wo_v, lo, nh * D))
        lo += nh * D
    wo_tail_cp = []
    for rows in wo_vpu_rows:
        wo_tail_cp.append(copy(wo_hbm, wo_v, lo, rows))
        lo += rows
    assert lo == H * D and sum(wo_vpu_rows) == D

    x_cp.start()
    for cp in wq_cp + wuk_cp:
        cp.start()
    for i in range(nck):
        ckv_copy(i).start()
    for cp in ffn_cp + wuv_cp + wo_cp + wo_tail_cp:
        cp.start()
    hook("start")

    ei = lax.broadcasted_iota(jnp.int32, (128, G), 0)
    ej = lax.broadcasted_iota(jnp.int32, (128, G), 1)
    e_v[...] = jnp.where(ej // H == ei, 1.0, 0.0).astype(_BF16)
    di = lax.broadcasted_iota(jnp.int32, (H, G), 0)
    dj = lax.broadcasted_iota(jnp.int32, (H, G), 1)
    diag = (dj % H) == di

    def expand(rows_bf16):
        ex = jnp.dot(rows_bf16, e_v[...], preferred_element_type=_F32)
        return jnp.where(diag, ex, 0.0).astype(_BF16)

    x_cp.wait()
    x = x_v[...].astype(_F32)
    mu = jnp.mean(x, axis=-1, keepdims=True)
    xc = x - mu
    var = jnp.mean(xc * xc, axis=-1, keepdims=True)
    xn = (xc / jnp.sqrt(var + eps)).astype(_BF16)
    xn_h = jnp.broadcast_to(xn, (H, M))

    aq = [expand(xn_h[:, a * 128:(a + 1) * 128]) for a in range(nq)]
    q = jnp.zeros((H, D), _F32)
    for a in range(nq):
        wq_cp[a].wait()
        hook("wq%d" % a)
        q = q + jnp.dot(aq[a], wq_v[a * G:(a + 1) * G, :], preferred_element_type=_F32)
    q = q.astype(_BF16)

    scale = D ** -0.5
    ql = []
    for a in range(nc):
        wuk_cp[a].wait()
        hook("wuk%d" % a)
        t = lax.dot_general(q, wuk_v[a * G:(a + 1) * G, :], _NT, preferred_element_type=_F32)
        t = jnp.where(diag, t * scale, 0.0).astype(_BF16)
        ql.append(lax.dot_general(t, e_v[...], _NT, preferred_element_type=_F32))
    q_lat = jnp.concatenate(ql, axis=-1).astype(_BF16)

    def step(i, carry):
        m_old, l_old, acc = carry
        ckv_copy(i).wait()
        side(J0 + i)
        kv = ckv_v[pl.ds(pl.multiple_of(i * TK, TK), TK), :]
        s = lax.dot_general(q_lat, kv, _NT, preferred_element_type=_F32)
        m_new = jnp.maximum(m_old, jnp.max(s, axis=-1, keepdims=True))
        alpha = jnp.exp(m_old - m_new)
        p = jnp.exp(s - m_new)
        l_new = alpha * l_old + jnp.sum(p, axis=-1, keepdims=True)
        acc = alpha * acc + jnp.dot(p.astype(_BF16), kv, preferred_element_type=_F32)
        return m_new, l_new, acc

    m0 = jnp.full((H, 1), -jnp.inf, _F32)
    l0 = jnp.zeros((H, 1), _F32)
    acc0 = jnp.zeros((H, C), _F32)
    _, l_fin, acc = lax.fori_loop(0, nck, step, (m0, l0, acc0))
    ctx_lat = (acc / l_fin).astype(_BF16)

    xn8 = jnp.broadcast_to(xn, (8, M))
    for cp in ffn_cp:
        cp.wait()
    hook("ffn")
    h1 = lax.dot_general(xn8, w1_v[...], _NT, preferred_element_type=_F32)
    h1 = _silu(h1).astype(_BF16)

    av = [expand(ctx_lat[:, a * 128:(a + 1) * 128]) for a in range(nc)]
    ctx = jnp.zeros((H, D), _F32)
    for a in range(nc):
        wuv_cp[a].wait()
        hook("wuv%d" % a)
        ctx = ctx + jnp.dot(av[a], wuv_v[a * G:(a + 1) * G, :], preferred_element_type=_F32)
    ctx = ctx.astype(_BF16).astype(_F32)

    row8 = lax.broadcasted_iota(jnp.int32, (8, D), 0)

    def head_lhs(h):
        grp = ctx[(h // 8) * 8:(h // 8) * 8 + 8, :]
        return jnp.where(row8 == (h % 8), grp, 0.0).astype(_BF16)

    eye = (lax.broadcasted_iota(jnp.int32, (D, D), 0)
           == lax.broadcasted_iota(jnp.int32, (D, D), 1))
    last = jnp.where(eye, jnp.broadcast_to(ctx[H - 1:H, :], (D, D)), 0.0).astype(_BF16)
    last_col = jnp.dot(last, jnp.ones((D, 128), _BF16), preferred_element_type=_F32)

    so8 = jnp.zeros((8, M), _F32)
    g = None
    h0 = 0
    for k, (cp, nh) in enumerate(zip(wo_cp, wo_mxu_heads)):
        lhs = jnp.concatenate([head_lhs(h) for h in range(h0, h0 + nh)], axis=-1)
        cp.wait()
        hook("wo%d" % k)
        so8 = so8 + jnp.dot(lhs, wo_v[h0 * D:(h0 + nh) * D, :], preferred_element_type=_F32)
        h0 += nh
        if "wo%d" % k == post_hooks[-1]:
            g = _silu(jnp.dot(h1, w2_v[...], preferred_element_type=_F32))[0:1]
    r0 = 0
    for cp, rows in zip(wo_tail_cp, wo_vpu_rows):
        coef = jnp.concatenate([last_col[r0:r0 + rows, :]] * (M // 128), axis=-1)
        cp.wait()
        w = wo_v[h0 * D + r0:h0 * D + r0 + rows, :].astype(_F32)
        prod = coef * w
        for r in range(0, rows, 8):
            so8 = so8 + prod[r:r + 8, :]
        r0 += rows
    s = jnp.sum(so8, axis=0, keepdims=True)

    o_ref[...] = (x + s * g).astype(o_ref.dtype)


def _kernel(*refs, n_sems, **kw):
    pl.run_scoped(lambda sems: _body(*refs, sems, **kw),
                  pltpu.SemaphoreType.DMA((n_sems,)))


def _forward(A_x, A_c_kv, A_w_q, A_w_uk, A_w_uv, A_w_o, B_w1, B_w2, *,
             TK=2048, stage_rows=48,
             pre_hooks=("start", "wq1", "wq3", "wuk1", "wuk3"),
             post_hooks=("ffn", "wuv1", "wuv3", "wo0"),
             wo_mxu_heads=(8, 8, 8, 4, 2, 1), wo_vpu_rows=(96, 32)):
    B, SQ, M = A_x.shape
    _, SK, C = A_c_kv.shape
    _, H, D = A_w_q.shape
    F = B_w1.shape[1]
    assert B == 1 and SQ == 1 and D == 128 and H == 32 and M % 128 == 0 and C % 128 == 0
    stage_slots = 3
    n_sems = (SK // TK + 2 * stage_slots + 3 + M // 128 + 2 * (C // 128)
              + len(wo_mxu_heads) + len(wo_vpu_rows))
    dt = A_x.dtype

    kernel = functools.partial(
        _kernel, n_sems=n_sems, H=H, D=D, M=M, C=C, SK=SK, TK=TK,
        wo_mxu_heads=wo_mxu_heads, wo_vpu_rows=wo_vpu_rows,
        pre_hooks=pre_hooks, post_hooks=post_hooks, eps=1e-5)
    any_spec = pl.BlockSpec(memory_space=pl.ANY)
    out = pl.pallas_call(
        kernel,
        in_specs=[any_spec] * 8,
        out_specs=pl.BlockSpec(memory_space=pltpu.VMEM),
        out_shape=jax.ShapeDtypeStruct((1, M), dt),
        scratch_shapes=[
            pltpu.VMEM((1, M), dt),
            pltpu.VMEM((SK, C), dt),
            pltpu.VMEM((M * H, D), dt),
            pltpu.VMEM((C * H, D), dt),
            pltpu.VMEM((C * H, D), dt),
            pltpu.VMEM((H * D, M), dt),
            pltpu.VMEM((F, M), dt),
            pltpu.VMEM((F, M), dt),
            pltpu.VMEM((128, 128 * H), _BF16),
            pltpu.SMEM((stage_slots, stage_rows, M), dt),
        ],
        compiler_params=pltpu.CompilerParams(vmem_limit_bytes=100 * 1024 * 1024),
    )(
        A_x.reshape(1, M),
        A_c_kv.reshape(SK, C),
        A_w_q.reshape(M * H, D),
        A_w_uk.reshape(C * H, D),
        A_w_uv.reshape(C * H, D),
        A_w_o.reshape(H * D, M),
        B_w1.T,
        B_w2,
    )
    return out.reshape(B, SQ, M)


@jax.jit
def pallas_recurrent_scan__compressed_kv_cla__dense_activation_silu__decode_kernel(
    A_x: jax.Array,
    A_c_kv: jax.Array,
    A_w_q: jax.Array,
    A_w_uk: jax.Array,
    A_w_uv: jax.Array,
    A_w_o: jax.Array,
    B_x: jax.Array,
    B_w1: jax.Array,
    B_w2: jax.Array,
):
    return _forward(A_x, A_c_kv, A_w_q, A_w_uk, A_w_uv, A_w_o, B_w1, B_w2)
```

```python
import functools

import jax
import jax.numpy as jnp
from jax import lax
import jax.experimental.pallas as pl
import jax.experimental.pallas.tpu as pltpu

_F32 = jnp.float32
_BF16 = jnp.bfloat16
_NT = (((1,), (1,)), ((), ()))


def _silu(v):
    return v / (1.0 + jnp.exp(-v))


def _body(x_hbm, ckv_hbm, wq_hbm, wuk_hbm, wuv_hbm, wo_hbm, w1_hbm, w2_hbm,
          o_ref,
          x_v, ckv_v, wq_v, wuk_v, wuv_v, wo_v, w1_v, w2_v, e_v, stage, sems,
          *, H, D, M, C, SK, TK, wo_mxu_rows, wo_vpu_rows, pre_hooks, post_hooks,
          side_lags, late_issue_step, eps):
    nck = SK // TK
    G = 128 * H
    nq = M // 128
    nc = C // 128

    n_sem = [0]

    def copy(src, dst, lo=None, rows=None):
        sem = sems.at[n_sem[0]]
        n_sem[0] += 1
        if lo is None:
            return pltpu.make_async_copy(src, dst, sem)
        return pltpu.make_async_copy(src.at[pl.ds(lo, rows)], dst.at[pl.ds(lo, rows)], sem)

    def ckv_copy(i):
        return pltpu.make_async_copy(ckv_hbm.at[pl.ds(i * TK, TK)],
                                     ckv_v.at[pl.ds(i * TK, TK)], sems.at[i])

    S, R, _ = stage.shape
    J0 = len(pre_hooks)
    L1, L2 = side_lags
    NS = J0 + nck + len(post_hooks) - L2
    assert S == L2 + 1 and J0 >= L2 and len(post_hooks) >= L2
    sem_h2s, sem_s2v = nck, nck + S

    def piece(j):
        return j * R if isinstance(j, int) else pl.multiple_of(j * R, 16)

    def h2s(j):
        return pltpu.make_async_copy(wo_hbm.at[pl.ds(piece(j), R)], stage.at[j % S],
                                     sems.at[sem_h2s + j % S])

    def s2v(j):
        return pltpu.make_async_copy(stage.at[j % S], wo_v.at[pl.ds(piece(j), R)],
                                     sems.at[sem_s2v + j % S])

    def side(j):
        static = isinstance(j, int)
        if not static or j < NS:
            h2s(j).start()
        if not static or L1 <= j < NS + L1:
            h2s(j - L1).wait()
            s2v(j - L1).start()
        if not static or L2 <= j < NS + L2:
            s2v(j - L2).wait()

    side_done = [0]

    def hook(name):
        for k, other in enumerate(pre_hooks):
            if other == name:
                side(k)
        for k, other in enumerate(post_hooks):
            if other == name:
                side(J0 + nck + k)
                side_done[0] = J0 + nck + k - L2 + 1

    n_sem[0] = nck + 2 * S
    x_cp = copy(x_hbm, x_v)
    wq_cp = [copy(wq_hbm, wq_v, a * G, G) for a in range(nq)]
    wuk_cp = [copy(wuk_hbm, wuk_v, a * G, G) for a in range(nc)]
    w1_cp = copy(w1_hbm, w1_v)
    w2_cp = copy(w2_hbm, w2_v)
    wuv_cp = [copy(wuv_hbm, wuv_v, a * G, G) for a in range(nc)]
    wo_first = H * D - sum(wo_mxu_rows) - sum(wo_vpu_rows) - NS * R
    wo_rows = (wo_first,) + tuple(wo_mxu_rows)
    assert wo_first > 0 and sum(wo_vpu_rows) == D
    wo_cp = []
    lo = NS * R
    for rows in wo_rows + tuple(wo_vpu_rows):
        wo_cp.append(copy(wo_hbm, wo_v, lo, rows))
        lo += rows

    x_cp.start()
    for cp in wq_cp + wuk_cp:
        cp.start()
    for i in range(nck):
        ckv_copy(i).start()
    hook("start")

    def issue_late():
        for cp in [w1_cp, w2_cp] + wuv_cp + wo_cp:
            cp.start()

    ei = lax.broadcasted_iota(jnp.int32, (128, G), 0)
    ej = lax.broadcasted_iota(jnp.int32, (128, G), 1)
    e_v[...] = jnp.where(ej // H == ei, 1.0, 0.0).astype(_BF16)
    di = lax.broadcasted_iota(jnp.int32, (H, G), 0)
    dj = lax.broadcasted_iota(jnp.int32, (H, G), 1)
    diag = (dj % H) == di

    def expand(rows_bf16):
        ex = jnp.dot(rows_bf16, e_v[...], preferred_element_type=_F32)
        return jnp.where(diag, ex, 0.0).astype(_BF16)

    x_cp.wait()
    x = x_v[...].astype(_F32)
    mu = jnp.mean(x, axis=-1, keepdims=True)
    xc = x - mu
    var = jnp.mean(xc * xc, axis=-1, keepdims=True)
    xn = (xc / jnp.sqrt(var + eps)).astype(_BF16)
    xn_h = jnp.broadcast_to(xn, (H, M))

    aq = [expand(xn_h[:, a * 128:(a + 1) * 128]) for a in range(nq)]
    q = jnp.zeros((H, D), _F32)
    for a in range(nq):
        wq_cp[a].wait()
        hook("wq%d" % a)
        q = q + jnp.dot(aq[a], wq_v[a * G:(a + 1) * G, :], preferred_element_type=_F32)
    q = q.astype(_BF16)

    scale = D ** -0.5
    ql = []
    for a in range(nc):
        wuk_cp[a].wait()
        hook("wuk%d" % a)
        t = lax.dot_general(q, wuk_v[a * G:(a + 1) * G, :], _NT, preferred_element_type=_F32)
        t = jnp.where(diag, t * scale, 0.0).astype(_BF16)
        ql.append(lax.dot_general(t, e_v[...], _NT, preferred_element_type=_F32))
    q_lat = jnp.concatenate(ql, axis=-1).astype(_BF16)

    def step(i, carry):
        m_old, l_old, acc = carry
        pl.when(i == late_issue_step)(issue_late)
        ckv_copy(i).wait()
        side(J0 + i)
        kv = ckv_v[pl.ds(pl.multiple_of(i * TK, TK), TK), :]
        s = lax.dot_general(q_lat, kv, _NT, preferred_element_type=_F32)
        m_new = jnp.maximum(m_old, jnp.max(s, axis=-1, keepdims=True))
        alpha = jnp.exp(m_old - m_new)
        p = jnp.exp(s - m_new)
        l_new = alpha * l_old + jnp.sum(p, axis=-1, keepdims=True)
        acc = alpha * acc + jnp.dot(p.astype(_BF16), kv, preferred_element_type=_F32)
        return m_new, l_new, acc

    m0 = jnp.full((H, 1), -jnp.inf, _F32)
    l0 = jnp.zeros((H, 1), _F32)
    acc0 = jnp.zeros((H, C), _F32)
    _, l_fin, acc = lax.fori_loop(0, nck, step, (m0, l0, acc0))
    ctx_lat = (acc / l_fin).astype(_BF16)

    xn8 = jnp.broadcast_to(xn, (8, M))
    w1_cp.wait()
    hook("w1")
    h1 = lax.dot_general(xn8, w1_v[...], _NT, preferred_element_type=_F32)
    h1 = _silu(h1).astype(_BF16)
    av = [expand(ctx_lat[:, a * 128:(a + 1) * 128]) for a in range(nc)]
    w2_cp.wait()
    hook("w2")
    g = _silu(jnp.dot(h1, w2_v[...], preferred_element_type=_F32))[0:1]

    ctx = jnp.zeros((H, D), _F32)
    for a in range(nc):
        wuv_cp[a].wait()
        hook("wuv%d" % a)
        ctx = ctx + jnp.dot(av[a], wuv_v[a * G:(a + 1) * G, :], preferred_element_type=_F32)
    ctx = ctx.astype(_BF16).astype(_F32)

    row8 = lax.broadcasted_iota(jnp.int32, (8, D), 0)
    lhs = jnp.concatenate(
        [jnp.where(row8 == (h % 8), ctx[(h // 8) * 8:(h // 8) * 8 + 8, :], 0.0)
         for h in range(H)], axis=-1).astype(_BF16)

    def wo_dot(lo, hi):
        return jnp.dot(lhs[:, lo:hi], wo_v[lo:hi, :], preferred_element_type=_F32)

    eye = (lax.broadcasted_iota(jnp.int32, (D, D), 0)
           == lax.broadcasted_iota(jnp.int32, (D, D), 1))
    last = jnp.where(eye, jnp.broadcast_to(ctx[H - 1:H, :], (D, D)), 0.0).astype(_BF16)
    last_col = jnp.dot(last, jnp.ones((D, 128), _BF16), preferred_element_type=_F32)

    side_used = (side_done[0] * R) // 128 * 128 if side_done[0] < NS else NS * R
    so8 = wo_dot(0, side_used)
    lo = NS * R
    for k, rows in enumerate(wo_rows):
        wo_cp[k].wait()
        hook("wo%d" % k)
        so8 = so8 + wo_dot(lo, lo + rows)
        lo += rows
        if side_done[0] == NS and side_used < NS * R:
            so8 = so8 + wo_dot(side_used, NS * R)
            side_used = NS * R
    assert side_used == NS * R
    r0 = 0
    for cp, rows in zip(wo_cp[len(wo_rows):], wo_vpu_rows):
        coef = jnp.concatenate([last_col[r0:r0 + rows, :]] * (M // 128), axis=-1)
        cp.wait()
        prod = coef * wo_v[lo + r0:lo + r0 + rows, :].astype(_F32)
        for r in range(0, rows, 8):
            so8 = so8 + prod[r:r + 8, :]
        r0 += rows
    s = jnp.sum(so8, axis=0, keepdims=True)

    o_ref[...] = (x + s * g).astype(o_ref.dtype)


def _kernel(*refs, n_sems, **kw):
    pl.run_scoped(lambda sems: _body(*refs, sems, **kw),
                  pltpu.SemaphoreType.DMA((n_sems,)))


def _forward(A_x, A_c_kv, A_w_q, A_w_uk, A_w_uv, A_w_o, B_w1, B_w2, *,
             TK=2048, stage_rows=64, side_lags=(1, 3), late_issue_step=10,
             pre_hooks=("start", "wq0", "wq2", "wuk0", "wuk2"),
             post_hooks=("w1", "wuv0", "wuv2", "wo0"),
             wo_mxu_rows=(1024, 512, 256, 128), wo_vpu_rows=(96, 32)):
    B, SQ, M = A_x.shape
    _, SK, C = A_c_kv.shape
    _, H, D = A_w_q.shape
    F = B_w1.shape[1]
    assert B == 1 and SQ == 1 and D == 128 and H == 32 and M % 128 == 0 and C % 128 == 0
    stage_slots = side_lags[1] + 1
    n_sems = (SK // TK + 2 * stage_slots + 4 + M // 128 + 2 * (C // 128)
              + len(wo_mxu_rows) + len(wo_vpu_rows))
    dt = A_x.dtype

    kernel = functools.partial(
        _kernel, n_sems=n_sems, H=H, D=D, M=M, C=C, SK=SK, TK=TK,
        wo_mxu_rows=wo_mxu_rows, wo_vpu_rows=wo_vpu_rows,
        pre_hooks=pre_hooks, post_hooks=post_hooks, side_lags=side_lags,
        late_issue_step=late_issue_step, eps=1e-5)
    any_spec = pl.BlockSpec(memory_space=pl.ANY)
    out = pl.pallas_call(
        kernel,
        in_specs=[any_spec] * 8,
        out_specs=pl.BlockSpec(memory_space=pltpu.VMEM),
        out_shape=jax.ShapeDtypeStruct((1, M), dt),
        scratch_shapes=[
            pltpu.VMEM((1, M), dt),
            pltpu.VMEM((SK, C), dt),
            pltpu.VMEM((M * H, D), dt),
            pltpu.VMEM((C * H, D), dt),
            pltpu.VMEM((C * H, D), dt),
            pltpu.VMEM((H * D, M), dt),
            pltpu.VMEM((F, M), dt),
            pltpu.VMEM((F, M), dt),
            pltpu.VMEM((128, 128 * H), _BF16),
            pltpu.SMEM((stage_slots, stage_rows, M), dt),
        ],
        compiler_params=pltpu.CompilerParams(vmem_limit_bytes=100 * 1024 * 1024),
    )(
        A_x.reshape(1, M),
        A_c_kv.reshape(SK, C),
        A_w_q.reshape(M * H, D),
        A_w_uk.reshape(C * H, D),
        A_w_uv.reshape(C * H, D),
        A_w_o.reshape(H * D, M),
        B_w1.T,
        B_w2,
    )
    return out.reshape(B, SQ, M)


@jax.jit
def pallas_recurrent_scan__compressed_kv_cla__dense_activation_silu__decode_kernel(
    A_x: jax.Array,
    A_c_kv: jax.Array,
    A_w_q: jax.Array,
    A_w_uk: jax.Array,
    A_w_uv: jax.Array,
    A_w_o: jax.Array,
    B_x: jax.Array,
    B_w1: jax.Array,
    B_w2: jax.Array,
):
    return _forward(A_x, A_c_kv, A_w_q, A_w_uk, A_w_uv, A_w_o, B_w1, B_w2)
```

```python
import functools

import jax
import jax.numpy as jnp
from jax import lax
import jax.experimental.pallas as pl
import jax.experimental.pallas.tpu as pltpu

_F32 = jnp.float32
_BF16 = jnp.bfloat16
_NT = (((1,), (1,)), ((), ()))


def _silu(v):
    return v / (1.0 + jnp.exp(-v))


def _body(x_hbm, ckv_hbm, wq_hbm, wuk_hbm, wuv_hbm, wo_hbm, w1_hbm, w2_hbm,
          o_ref,
          x_v, ckv_v, wq_v, wuk_v, wuv_v, wo_v, w1_v, w2_v, e_v, stage, sems,
          *, H, D, M, C, SK, TK, wo_mxu_rows, wo_vpu_rows, pre_hooks, post_hooks,
          side_lags, late_issue_step, eps):
    nck = SK // TK
    G = 128 * H
    nq = M // 128
    nc = C // 128

    n_sem = [0]

    def copy(src, dst, lo=None, rows=None):
        sem = sems.at[n_sem[0]]
        n_sem[0] += 1
        if lo is None:
            return pltpu.make_async_copy(src, dst, sem)
        return pltpu.make_async_copy(src.at[pl.ds(lo, rows)], dst.at[pl.ds(lo, rows)], sem)

    def ckv_copy(i):
        return pltpu.make_async_copy(ckv_hbm.at[pl.ds(i * TK, TK)],
                                     ckv_v.at[pl.ds(i * TK, TK)], sems.at[i])

    S, R, _ = stage.shape
    J0 = len(pre_hooks)
    L1, L2 = side_lags
    NS = J0 + nck + len(post_hooks) - L2
    assert S == L2 + 1 and J0 >= L2 and len(post_hooks) >= L2
    sem_h2s, sem_s2v = nck, nck + S

    def piece(j):
        return j * R if isinstance(j, int) else pl.multiple_of(j * R, 16)

    def h2s(j):
        return pltpu.make_async_copy(wo_hbm.at[pl.ds(piece(j), R)], stage.at[j % S],
                                     sems.at[sem_h2s + j % S])

    def s2v(j):
        return pltpu.make_async_copy(stage.at[j % S], wo_v.at[pl.ds(piece(j), R)],
                                     sems.at[sem_s2v + j % S])

    def side(j):
        static = isinstance(j, int)
        if not static or j < NS:
            h2s(j).start()
        if not static or L1 <= j < NS + L1:
            h2s(j - L1).wait()
            s2v(j - L1).start()
        if not static or L2 <= j < NS + L2:
            s2v(j - L2).wait()

    side_done = [0]

    def hook(name):
        for k, other in enumerate(pre_hooks):
            if other == name:
                side(k)
        for k, other in enumerate(post_hooks):
            if other == name:
                side(J0 + nck + k)
                side_done[0] = J0 + nck + k - L2 + 1

    n_sem[0] = nck + 2 * S
    x_cp = copy(x_hbm, x_v)
    wq_cp = [copy(wq_hbm, wq_v, a * G, G) for a in range(nq)]
    wuk_cp = [copy(wuk_hbm, wuk_v, a * G, G) for a in range(nc)]
    w1_cp = copy(w1_hbm, w1_v)
    w2_cp = copy(w2_hbm, w2_v)
    wuv_cp = [copy(wuv_hbm, wuv_v, a * G, G) for a in range(nc)]
    wo_first = H * D - sum(wo_mxu_rows) - sum(wo_vpu_rows) - NS * R
    wo_rows = (wo_first,) + tuple(wo_mxu_rows)
    assert wo_first > 0 and sum(wo_vpu_rows) % D == 0
    wo_cp = []
    lo = NS * R
    for rows in wo_rows + tuple(wo_vpu_rows):
        wo_cp.append(copy(wo_hbm, wo_v, lo, rows))
        lo += rows

    x_cp.start()
    for cp in wq_cp + wuk_cp:
        cp.start()
    for i in range(nck):
        ckv_copy(i).start()
    hook("start")

    def issue_late():
        for cp in [w1_cp, w2_cp] + wuv_cp + wo_cp:
            cp.start()

    ei = lax.broadcasted_iota(jnp.int32, (128, G), 0)
    ej = lax.broadcasted_iota(jnp.int32, (128, G), 1)
    e_v[...] = jnp.where(ej // H == ei, 1.0, 0.0).astype(_BF16)
    di = lax.broadcasted_iota(jnp.int32, (H, G), 0)
    dj = lax.broadcasted_iota(jnp.int32, (H, G), 1)
    diag = (dj % H) == di

    def expand(rows_bf16):
        ex = jnp.dot(rows_bf16, e_v[...], preferred_element_type=_F32)
        return jnp.where(diag, ex, 0.0).astype(_BF16)

    x_cp.wait()
    x = x_v[...].astype(_F32)
    mu = jnp.mean(x, axis=-1, keepdims=True)
    xc = x - mu
    var = jnp.mean(xc * xc, axis=-1, keepdims=True)
    xn = (xc / jnp.sqrt(var + eps)).astype(_BF16)
    xn_h = jnp.broadcast_to(xn, (H, M))

    aq = [expand(xn_h[:, a * 128:(a + 1) * 128]) for a in range(nq)]
    q = jnp.zeros((H, D), _F32)
    for a in range(nq):
        wq_cp[a].wait()
        hook("wq%d" % a)
        q = q + jnp.dot(aq[a], wq_v[a * G:(a + 1) * G, :], preferred_element_type=_F32)
    q = q.astype(_BF16)

    scale = D ** -0.5
    ql = []
    for a in range(nc):
        wuk_cp[a].wait()
        hook("wuk%d" % a)
        t = lax.dot_general(q, wuk_v[a * G:(a + 1) * G, :], _NT, preferred_element_type=_F32)
        t = jnp.where(diag, t * scale, 0.0).astype(_BF16)
        ql.append(lax.dot_general(t, e_v[...], _NT, preferred_element_type=_F32))
    q_lat = jnp.concatenate(ql, axis=-1).astype(_BF16)

    def step(i, carry):
        m_old, l_old, acc = carry
        pl.when(i == late_issue_step)(issue_late)
        ckv_copy(i).wait()
        side(J0 + i)
        kv = ckv_v[pl.ds(pl.multiple_of(i * TK, TK), TK), :]
        s = lax.dot_general(q_lat, kv, _NT, preferred_element_type=_F32)
        m_new = jnp.maximum(m_old, jnp.max(s, axis=-1, keepdims=True))
        alpha = jnp.exp(m_old - m_new)
        p = jnp.exp(s - m_new)
        l_new = alpha * l_old + jnp.sum(p, axis=-1, keepdims=True)
        acc = alpha * acc + jnp.dot(p.astype(_BF16), kv, preferred_element_type=_F32)
        return m_new, l_new, acc

    m0 = jnp.full((H, 1), -jnp.inf, _F32)
    l0 = jnp.zeros((H, 1), _F32)
    acc0 = jnp.zeros((H, C), _F32)
    _, l_fin, acc = lax.fori_loop(0, nck, step, (m0, l0, acc0))
    ctx_lat = (acc / l_fin).astype(_BF16)

    xn8 = jnp.broadcast_to(xn, (8, M))
    w1_cp.wait()
    hook("w1")
    h1 = lax.dot_general(xn8, w1_v[...], _NT, preferred_element_type=_F32)
    h1 = _silu(h1).astype(_BF16)
    av = [expand(ctx_lat[:, a * 128:(a + 1) * 128]) for a in range(nc)]
    w2_cp.wait()
    hook("w2")
    g = _silu(jnp.dot(h1, w2_v[...], preferred_element_type=_F32))[0:1]

    ctx = jnp.zeros((H, D), _F32)
    for a in range(nc):
        wuv_cp[a].wait()
        hook("wuv%d" % a)
        ctx = ctx + jnp.dot(av[a], wuv_v[a * G:(a + 1) * G, :], preferred_element_type=_F32)
    ctx = ctx.astype(_BF16).astype(_F32)

    row8 = lax.broadcasted_iota(jnp.int32, (8, D), 0)
    lhs = jnp.concatenate(
        [jnp.where(row8 == (h % 8), ctx[(h // 8) * 8:(h // 8) * 8 + 8, :], 0.0)
         for h in range(H)], axis=-1).astype(_BF16)

    def wo_dot(lo, hi):
        return jnp.dot(lhs[:, lo:hi], wo_v[lo:hi, :], preferred_element_type=_F32)

    eye = (lax.broadcasted_iota(jnp.int32, (D, D), 0)
           == lax.broadcasted_iota(jnp.int32, (D, D), 1))
    last = jnp.concatenate(
        [jnp.where(eye, jnp.broadcast_to(ctx[h:h + 1, :], (D, D)), 0.0).astype(_BF16)
         for h in range(H - sum(wo_vpu_rows) // D, H)], axis=0)
    last_col = jnp.dot(last, jnp.ones((D, 128), _BF16), preferred_element_type=_F32)
    x8 = jnp.broadcast_to(x, (8, M))

    side_used = (side_done[0] * R) // 128 * 128 if side_done[0] < NS else NS * R
    so8 = wo_dot(0, side_used)
    lo = NS * R
    for k, rows in enumerate(wo_rows):
        wo_cp[k].wait()
        hook("wo%d" % k)
        so8 = so8 + wo_dot(lo, lo + rows)
        lo += rows
        if side_done[0] == NS and side_used < NS * R:
            so8 = so8 + wo_dot(side_used, NS * R)
            side_used = NS * R
    assert side_used == NS * R
    r0 = 0
    for cp, rows in zip(wo_cp[len(wo_rows):], wo_vpu_rows):
        coef = jnp.concatenate([last_col[r0:r0 + rows, :]] * (M // 128), axis=-1)
        cp.wait()
        prod = coef * wo_v[lo + r0:lo + r0 + rows, :].astype(_F32)
        for r in range(0, rows, 8):
            so8 = so8 + prod[r:r + 8, :]
        r0 += rows
    s = jnp.sum(so8, axis=0, keepdims=True)

    o_ref[...] = (x8[0:1] + s * g).astype(o_ref.dtype)


def _kernel(*refs, n_sems, **kw):
    pl.run_scoped(lambda sems: _body(*refs, sems, **kw),
                  pltpu.SemaphoreType.DMA((n_sems,)))


def _forward(A_x, A_c_kv, A_w_q, A_w_uk, A_w_uv, A_w_o, B_w1, B_w2, *,
             TK=2048, stage_rows=64, side_lags=(3, 5), late_issue_step=12,
             pre_hooks=("start", "start", "start", "wq1", "wq3", "wuk1", "wuk3"),
             post_hooks=("w1", "wuv0", "wuv2", "wuv3", "wo0", "wo1"),
             wo_mxu_rows=(1024, 512), wo_vpu_rows=(256, 128, 64, 48, 16)):
    B, SQ, M = A_x.shape
    _, SK, C = A_c_kv.shape
    _, H, D = A_w_q.shape
    F = B_w1.shape[1]
    assert B == 1 and SQ == 1 and D == 128 and H == 32 and M % 128 == 0 and C % 128 == 0
    stage_slots = side_lags[1] + 1
    n_sems = (SK // TK + 2 * stage_slots + 4 + M // 128 + 2 * (C // 128)
              + len(wo_mxu_rows) + len(wo_vpu_rows))
    dt = A_x.dtype

    kernel = functools.partial(
        _kernel, n_sems=n_sems, H=H, D=D, M=M, C=C, SK=SK, TK=TK,
        wo_mxu_rows=wo_mxu_rows, wo_vpu_rows=wo_vpu_rows,
        pre_hooks=pre_hooks, post_hooks=post_hooks, side_lags=side_lags,
        late_issue_step=late_issue_step, eps=1e-5)
    any_spec = pl.BlockSpec(memory_space=pl.ANY)
    out = pl.pallas_call(
        kernel,
        in_specs=[any_spec] * 8,
        out_specs=pl.BlockSpec(memory_space=pltpu.VMEM),
        out_shape=jax.ShapeDtypeStruct((1, M), dt),
        scratch_shapes=[
            pltpu.VMEM((1, M), dt),
            pltpu.VMEM((SK, C), dt),
            pltpu.VMEM((M * H, D), dt),
            pltpu.VMEM((C * H, D), dt),
            pltpu.VMEM((C * H, D), dt),
            pltpu.VMEM((H * D, M), dt),
            pltpu.VMEM((F, M), dt),
            pltpu.VMEM((F, M), dt),
            pltpu.VMEM((128, 128 * H), _BF16),
            pltpu.SMEM((stage_slots, stage_rows, M), dt),
        ],
        compiler_params=pltpu.CompilerParams(vmem_limit_bytes=100 * 1024 * 1024),
    )(
        A_x.reshape(1, M),
        A_c_kv.reshape(SK, C),
        A_w_q.reshape(M * H, D),
        A_w_uk.reshape(C * H, D),
        A_w_uv.reshape(C * H, D),
        A_w_o.reshape(H * D, M),
        B_w1.T,
        B_w2,
    )
    return out.reshape(B, SQ, M)


@jax.jit
def pallas_recurrent_scan__compressed_kv_cla__dense_activation_silu__decode_kernel(
    A_x: jax.Array,
    A_c_kv: jax.Array,
    A_w_q: jax.Array,
    A_w_uk: jax.Array,
    A_w_uv: jax.Array,
    A_w_o: jax.Array,
    B_x: jax.Array,
    B_w1: jax.Array,
    B_w2: jax.Array,
):
    return _forward(A_x, A_c_kv, A_w_q, A_w_uk, A_w_uv, A_w_o, B_w1, B_w2)
```

```python
import functools

import jax
import jax.numpy as jnp
from jax import lax
import jax.experimental.pallas as pl
import jax.experimental.pallas.tpu as pltpu

_F32 = jnp.float32
_BF16 = jnp.bfloat16
_NT = (((1,), (1,)), ((), ()))


def _silu(v):
    return v / (1.0 + jnp.exp(-v))


def _body(x_hbm, ckv_hbm, wq_hbm, wuk_hbm, wuv_hbm, wo_hbm, w1_hbm, w2_hbm,
          o_ref,
          x_v, ckv_v, wq_v, wuk_v, wuv_v, wo_v, w1_v, w2_v, e_v, stage, sems,
          *, H, D, M, C, SK, TK, wo_mxu_rows, wo_vpu_rows, pre_hooks, post_hooks,
          side_lags, late_issue_step, eps):
    nck = SK // TK
    G = 128 * H
    nq = M // 128
    nc = C // 128

    n_sem = [0]

    def copy(src, dst, lo=None, rows=None):
        sem = sems.at[n_sem[0]]
        n_sem[0] += 1
        if lo is None:
            return pltpu.make_async_copy(src, dst, sem)
        return pltpu.make_async_copy(src.at[pl.ds(lo, rows)], dst.at[pl.ds(lo, rows)], sem)

    def ckv_copy(i):
        return pltpu.make_async_copy(ckv_hbm.at[:, i], ckv_v.at[i], sems.at[i])

    S, R, _ = stage.shape
    J0 = len(pre_hooks)
    L1, L2 = side_lags
    NS = J0 + nck + len(post_hooks) - L2
    assert S == L2 + 1 and J0 >= L2 and len(post_hooks) >= L2
    sem_h2s, sem_s2v = nck, nck + S

    def piece(j):
        return j * R if isinstance(j, int) else pl.multiple_of(j * R, 16)

    def h2s(j):
        return pltpu.make_async_copy(wo_hbm.at[pl.ds(piece(j), R)], stage.at[j % S],
                                     sems.at[sem_h2s + j % S])

    def s2v(j):
        return pltpu.make_async_copy(stage.at[j % S], wo_v.at[pl.ds(piece(j), R)],
                                     sems.at[sem_s2v + j % S])

    def side(j):
        static = isinstance(j, int)
        if not static or j < NS:
            h2s(j).start()
        if not static or L1 <= j < NS + L1:
            h2s(j - L1).wait()
            s2v(j - L1).start()
        if not static or L2 <= j < NS + L2:
            s2v(j - L2).wait()

    side_done = [0]

    def hook(name):
        for k, other in enumerate(pre_hooks):
            if other == name:
                side(k)
        for k, other in enumerate(post_hooks):
            if other == name:
                side(J0 + nck + k)
                side_done[0] = J0 + nck + k - L2 + 1

    n_sem[0] = nck + 2 * S
    x_cp = copy(x_hbm, x_v)
    wq_cp = [copy(wq_hbm, wq_v, a * G, G) for a in range(nq)]
    wuk_cp = [copy(wuk_hbm, wuk_v, a * G, G) for a in range(nc)]
    w1_cp = copy(w1_hbm, w1_v)
    w2_cp = copy(w2_hbm, w2_v)
    wuv_cp = [copy(wuv_hbm, wuv_v, a * G, G) for a in range(nc)]
    wo_first = H * D - sum(wo_mxu_rows) - sum(wo_vpu_rows) - NS * R
    wo_rows = (wo_first,) + tuple(wo_mxu_rows)
    assert wo_first > 0 and sum(wo_vpu_rows) % D == 0
    wo_cp = []
    lo = NS * R
    for rows in wo_rows + tuple(wo_vpu_rows):
        wo_cp.append(copy(wo_hbm, wo_v, lo, rows))
        lo += rows

    x_cp.start()
    for cp in wq_cp + wuk_cp:
        cp.start()
    for i in range(nck):
        ckv_copy(i).start()
    hook("start")

    def issue_late():
        for cp in [w1_cp, w2_cp] + wuv_cp + wo_cp:
            cp.start()

    ei = lax.broadcasted_iota(jnp.int32, (128, G), 0)
    ej = lax.broadcasted_iota(jnp.int32, (128, G), 1)
    e_v[...] = jnp.where(ej // H == ei, 1.0, 0.0).astype(_BF16)
    di = lax.broadcasted_iota(jnp.int32, (H, G), 0)
    dj = lax.broadcasted_iota(jnp.int32, (H, G), 1)
    diag = (dj % H) == di

    def expand(rows_bf16):
        ex = jnp.dot(rows_bf16, e_v[...], preferred_element_type=_F32)
        return jnp.where(diag, ex, 0.0).astype(_BF16)

    x_cp.wait()
    x = x_v[...].astype(_F32)
    mu = jnp.mean(x, axis=-1, keepdims=True)
    xc = x - mu
    var = jnp.mean(xc * xc, axis=-1, keepdims=True)
    xn = (xc / jnp.sqrt(var + eps)).astype(_BF16)
    xn_h = jnp.broadcast_to(xn, (H, M))

    aq = [expand(xn_h[:, a * 128:(a + 1) * 128]) for a in range(nq)]
    q = jnp.zeros((H, D), _F32)
    for a in range(nq):
        wq_cp[a].wait()
        hook("wq%d" % a)
        q = q + jnp.dot(aq[a], wq_v[a * G:(a + 1) * G, :], preferred_element_type=_F32)
    q = q.astype(_BF16)

    scale = D ** -0.5
    ql = []
    for a in range(nc):
        wuk_cp[a].wait()
        hook("wuk%d" % a)
        t = lax.dot_general(q, wuk_v[a * G:(a + 1) * G, :], _NT, preferred_element_type=_F32)
        t = jnp.where(diag, t * scale, 0.0).astype(_BF16)
        ql.append(lax.dot_general(t, e_v[...], _NT, preferred_element_type=_F32))
    q_lat = jnp.concatenate(ql, axis=-1).astype(_BF16)

    def step(i, carry):
        m_old, l_old, acc = carry
        pl.when(i == late_issue_step)(issue_late)
        ckv_copy(i).wait()
        side(J0 + i)
        kv = ckv_v[i].reshape(TK, C)
        s = lax.dot_general(q_lat, kv, _NT, preferred_element_type=_F32)
        m_new = jnp.maximum(m_old, jnp.max(s, axis=-1, keepdims=True))
        alpha = jnp.exp(m_old - m_new)
        p = jnp.exp(s - m_new)
        l_new = alpha * l_old + jnp.sum(p, axis=-1, keepdims=True)
        acc = alpha * acc + jnp.dot(p.astype(_BF16), kv, preferred_element_type=_F32)
        return m_new, l_new, acc

    m0 = jnp.full((H, 1), -jnp.inf, _F32)
    l0 = jnp.zeros((H, 1), _F32)
    acc0 = jnp.zeros((H, C), _F32)
    _, l_fin, acc = lax.fori_loop(0, nck, step, (m0, l0, acc0))
    ctx_lat = (acc / l_fin).astype(_BF16)

    xn8 = jnp.broadcast_to(xn, (8, M))
    w1_cp.wait()
    hook("w1")
    h1 = lax.dot_general(xn8, w1_v[...], _NT, preferred_element_type=_F32)
    h1 = _silu(h1).astype(_BF16)
    av = [expand(ctx_lat[:, a * 128:(a + 1) * 128]) for a in range(nc)]
    w2_cp.wait()
    hook("w2")
    g = _silu(jnp.dot(h1, w2_v[...], preferred_element_type=_F32))[0:1]

    ctx = jnp.zeros((H, D), _F32)
    for a in range(nc):
        wuv_cp[a].wait()
        hook("wuv%d" % a)
        ctx = ctx + jnp.dot(av[a], wuv_v[a * G:(a + 1) * G, :], preferred_element_type=_F32)
    ctx = ctx.astype(_BF16).astype(_F32)

    row8 = lax.broadcasted_iota(jnp.int32, (8, D), 0)
    lhs = jnp.concatenate(
        [jnp.where(row8 == (h % 8), ctx[(h // 8) * 8:(h // 8) * 8 + 8, :], 0.0)
         for h in range(H)], axis=-1).astype(_BF16)

    def wo_dot(lo, hi):
        return jnp.dot(lhs[:, lo:hi], wo_v[lo:hi, :], preferred_element_type=_F32)

    eye = (lax.broadcasted_iota(jnp.int32, (D, D), 0)
           == lax.broadcasted_iota(jnp.int32, (D, D), 1))
    last = jnp.concatenate(
        [jnp.where(eye, jnp.broadcast_to(ctx[h:h + 1, :], (D, D)), 0.0).astype(_BF16)
         for h in range(H - sum(wo_vpu_rows) // D, H)], axis=0)
    last_col = jnp.dot(last, jnp.ones((D, 128), _BF16), preferred_element_type=_F32)
    x8 = jnp.broadcast_to(x, (8, M))

    side_used = (side_done[0] * R) // 128 * 128 if side_done[0] < NS else NS * R
    so8 = wo_dot(0, side_used)
    lo = NS * R
    for k, rows in enumerate(wo_rows):
        wo_cp[k].wait()
        hook("wo%d" % k)
        so8 = so8 + wo_dot(lo, lo + rows)
        lo += rows
        if side_done[0] == NS and side_used < NS * R:
            so8 = so8 + wo_dot(side_used, NS * R)
            side_used = NS * R
    assert side_used == NS * R
    r0 = 0
    for cp, rows in zip(wo_cp[len(wo_rows):], wo_vpu_rows):
        coef = jnp.concatenate([last_col[r0:r0 + rows, :]] * (M // 128), axis=-1)
        cp.wait()
        prod = coef * wo_v[lo + r0:lo + r0 + rows, :].astype(_F32)
        for r in range(0, rows, 8):
            so8 = so8 + prod[r:r + 8, :]
        r0 += rows
    s = jnp.sum(so8, axis=0, keepdims=True)

    o_ref[...] = (x8[0:1] + s * g).astype(o_ref.dtype)


def _kernel(*refs, n_sems, **kw):
    pl.run_scoped(lambda sems: _body(*refs, sems, **kw),
                  pltpu.SemaphoreType.DMA((n_sems,)))


def _forward(A_x, A_c_kv, A_w_q, A_w_uk, A_w_uv, A_w_o, B_w1, B_w2, *,
             TK=2048, ckv_run=32, stage_rows=64, side_lags=(3, 5), late_issue_step=12,
             pre_hooks=("start", "start", "start", "wq1", "wq3", "wuk1", "wuk3"),
             post_hooks=("w1", "wuv0", "wuv2", "wuv3", "wo0", "wo1"),
             wo_mxu_rows=(1024, 512), wo_vpu_rows=(256, 128, 64, 48, 16)):
    B, SQ, M = A_x.shape
    _, SK, C = A_c_kv.shape
    _, H, D = A_w_q.shape
    F = B_w1.shape[1]
    assert B == 1 and SQ == 1 and D == 128 and H == 32 and M % 128 == 0 and C % 128 == 0
    stage_slots = side_lags[1] + 1
    n_sems = (SK // TK + 2 * stage_slots + 4 + M // 128 + 2 * (C // 128)
              + len(wo_mxu_rows) + len(wo_vpu_rows))
    dt = A_x.dtype

    kernel = functools.partial(
        _kernel, n_sems=n_sems, H=H, D=D, M=M, C=C, SK=SK, TK=TK,
        wo_mxu_rows=wo_mxu_rows, wo_vpu_rows=wo_vpu_rows,
        pre_hooks=pre_hooks, post_hooks=post_hooks, side_lags=side_lags,
        late_issue_step=late_issue_step, eps=1e-5)
    any_spec = pl.BlockSpec(memory_space=pl.ANY)
    out = pl.pallas_call(
        kernel,
        in_specs=[any_spec] * 8,
        out_specs=pl.BlockSpec(memory_space=pltpu.VMEM),
        out_shape=jax.ShapeDtypeStruct((1, M), dt),
        scratch_shapes=[
            pltpu.VMEM((1, M), dt),
            pltpu.VMEM((SK // TK, TK // ckv_run, ckv_run, C), dt),
            pltpu.VMEM((M * H, D), dt),
            pltpu.VMEM((C * H, D), dt),
            pltpu.VMEM((C * H, D), dt),
            pltpu.VMEM((H * D, M), dt),
            pltpu.VMEM((F, M), dt),
            pltpu.VMEM((F, M), dt),
            pltpu.VMEM((128, 128 * H), _BF16),
            pltpu.SMEM((stage_slots, stage_rows, M), dt),
        ],
        compiler_params=pltpu.CompilerParams(vmem_limit_bytes=100 * 1024 * 1024),
    )(
        A_x.reshape(1, M),
        A_c_kv.reshape(TK // ckv_run, SK // TK, ckv_run, C),
        A_w_q.reshape(M * H, D),
        A_w_uk.reshape(C * H, D),
        A_w_uv.reshape(C * H, D),
        A_w_o.reshape(H * D, M),
        B_w1.T,
        B_w2,
    )
    return out.reshape(B, SQ, M)


@jax.jit
def pallas_recurrent_scan__compressed_kv_cla__dense_activation_silu__decode_kernel(
    A_x: jax.Array,
    A_c_kv: jax.Array,
    A_w_q: jax.Array,
    A_w_uk: jax.Array,
    A_w_uv: jax.Array,
    A_w_o: jax.Array,
    B_x: jax.Array,
    B_w1: jax.Array,
    B_w2: jax.Array,
):
    return _forward(A_x, A_c_kv, A_w_q, A_w_uk, A_w_uv, A_w_o, B_w1, B_w2)
```

```python
import functools

import jax
import jax.numpy as jnp
from jax import lax
import jax.experimental.pallas as pl
import jax.experimental.pallas.tpu as pltpu

_F32 = jnp.float32
_BF16 = jnp.bfloat16
_NT = (((1,), (1,)), ((), ()))
_LO = 1
_HG = 16


def _silu(v):
    return v / (1.0 + jnp.exp(-v))


def _body(x_hbm, ckv_hbm, wq_hbm, wuk_hbm, wuv_hbm, wo_hbm, w1_hbm, w2_hbm,
          o_ref,
          x_v, arena, wq_v, wuk_v, wuv_v, e_v, junk, sems,
          *, H, D, M, C, TK, n_a, ffn_split, wo_piece, wo_mxu_rows, wo_vpu_rows, pre_bursts, spin_pre, spin_loop,
          qk_split, pv_split, post_bursts, spin_post, eps):
    NB, nck, RUN, _ = ckv_hbm.shape
    NS, NP, MR, NG, _, _ = wq_hbm.shape
    PB = 4
    NBLK = NP // PB
    BW = PB * MR * _HG
    EW = 128 * _HG
    FB = w1_hbm.shape[0]
    B1 = nck * NB
    B2 = B1 + FB
    BO = B2 + FB
    n_b = nck - n_a

    n_sem = [nck]

    def new_sem():
        n_sem[0] += 1
        return sems.at[n_sem[0] - 1]

    def ckv_copy(i):
        return pltpu.make_async_copy(ckv_hbm.at[:, i], arena.at[pl.ds(i * NB, NB)], sems.at[i])

    sem_w1, sem_w2, sem_wuv, sem_wo, sem_wo2 = (new_sem() for _ in range(5))

    def spin(n, t):
        return lax.fori_loop(0, n, lambda i, t: t * 5 + i, t)

    PV = 2
    NV = C // PV
    BV = (NV - sum(pre_bursts)) // nck
    assert sum(pre_bursts) + BV * nck == NV

    def wuv_burst(k0, n, nspin, t):
        def body(u, t):
            o = (k0 + u) * PV
            pltpu.make_async_copy(wuv_hbm.at[pl.ds(o, PV)], wuv_v.at[pl.ds(o, PV)], sem_wuv).start()
            return spin(nspin, t)
        return lax.fori_loop(0, n, body, t)

    npin = 1 + len(qk_split) + len(pv_split)
    assert npin % 2 == 0
    fb = npin // 2 - ffn_split
    ffn_hi = fb * n_a
    assert ffn_hi <= FB
    plan = ([(b, h * (RUN // 2), RUN // 2) for b in range(ffn_split) for h in (0, 1)]
            + [(b, 0, RUN) for b in range(ffn_split, fb)])

    def ffn_pin(i, slot):
        src, base, sem = ((w1_hbm, B1, sem_w1), (w2_hbm, B2, sem_w2))[slot % 2]
        b, r0, rows = plan[slot // 2]
        k = i * fb + b
        pltpu.make_async_copy(src.at[k, pl.ds(r0, rows)], arena.at[base + k, pl.ds(r0, rows)], sem).start()

    ppb = RUN // wo_piece

    def wo_inj(k, sem):
        r = pl.ds(pl.multiple_of((k % ppb) * wo_piece, wo_piece), wo_piece)
        pltpu.make_async_copy(wo_hbm.at[k // ppb, r], arena.at[BO + k // ppb, r], sem).start()

    def wo_pin(i, slot):
        wo_inj((i - n_a) * npin + slot, sem_wo)

    wo_hi = n_b * npin * wo_piece
    wo_hi2 = sum(post_bursts) * wo_piece
    assert wo_hi % RUN == 0 and wo_hi2 % RUN == 0

    def wo_slice(ref, base, lo, rows):
        if lo % RUN == 0 and rows % RUN == 0:
            return ref.at[pl.ds(base + lo // RUN, rows // RUN)]
        assert lo // RUN == (lo + rows - 1) // RUN
        return ref.at[base + lo // RUN, pl.ds(lo % RUN, rows)]

    def wo_rows_val(lo, rows):
        return wo_slice(arena, BO, lo, rows)[...].reshape(rows, M)

    x_cp = pltpu.make_async_copy(x_hbm, x_v, new_sem())
    wq_cp = [pltpu.make_async_copy(wq_hbm.at[:, p], wq_v.at[:, p], new_sem()) for p in range(NP)]
    wuk_cp = [pltpu.make_async_copy(wuk_hbm.at[:, p], wuk_v.at[:, p], new_sem()) for p in range(NP)]
    ffn_cp = [pltpu.make_async_copy(src.at[pl.ds(ffn_hi, FB - ffn_hi)],
                                    arena.at[pl.ds(base + ffn_hi, FB - ffn_hi)], new_sem())
              for src, base in ((w1_hbm, B1), (w2_hbm, B2))] if ffn_hi < FB else []
    wo_lo0 = wo_hi + wo_hi2
    wo_rows = (H * D - wo_lo0 - sum(wo_mxu_rows) - sum(wo_vpu_rows),) + tuple(wo_mxu_rows)
    assert wo_rows[0] > 0
    wo_cp = []
    lo = wo_lo0
    for rows in wo_rows + tuple(wo_vpu_rows):
        wo_cp.append(pltpu.make_async_copy(wo_slice(wo_hbm, 0, lo, rows), wo_slice(arena, BO, lo, rows), new_sem()))
        lo += rows

    queue = [x_cp] + wq_cp + wuk_cp + ffn_cp + [ckv_copy(i) for i in range(nck)]
    issued = [0]

    def issue(n):
        for cp in queue[issued[0]:issued[0] + n]:
            cp.start(priority=_LO)
        issued[0] = min(len(queue), issued[0] + n)

    issue(24)

    pre = [0, 0, jnp.int32(1)]

    def pre_burst():
        n = pre_bursts[pre[0]]
        if n:
            pre[2] = wuv_burst(pre[1], n, spin_pre, pre[2])
        pre[0] += 1
        pre[1] += n

    ei = lax.broadcasted_iota(jnp.int32, (128, EW), 0)
    ej = lax.broadcasted_iota(jnp.int32, (128, EW), 1)
    e_v[...] = jnp.where(ej // _HG == ei, 1.0, 0.0).astype(_BF16)

    def diag(rows, cols):
        di = lax.broadcasted_iota(jnp.int32, (rows, cols), 0)
        dj = lax.broadcasted_iota(jnp.int32, (rows, cols), 1)
        return (dj % _HG) == (di % _HG)

    def expand(v):
        R, K = v.shape
        st = jnp.concatenate([v[:, a * 128:(a + 1) * 128] for a in range(K // 128)], axis=0)
        ex = jnp.dot(st, e_v[...], preferred_element_type=_F32)
        ex = jnp.where(diag(st.shape[0], EW), ex, 0.0).astype(_BF16)
        return jnp.concatenate([ex[a * R:(a + 1) * R] for a in range(K // 128)], axis=-1)

    pre_burst()
    x_cp.wait()
    x = x_v[...].astype(_F32)
    mu = jnp.mean(x, axis=-1, keepdims=True)
    xc = x - mu
    var = jnp.mean(xc * xc, axis=-1, keepdims=True)
    xn = (xc / jnp.sqrt(var + eps)).astype(_BF16)
    aq = expand(jnp.broadcast_to(xn, (_HG, M)))

    def wblock(ref, b, g):
        return ref[:, b * PB:(b + 1) * PB, :, g].reshape(NS * BW, D)

    SW = NP * MR * _HG
    qg = [jnp.zeros((_HG, D), _F32) for _ in range(NG)]
    for b in range(NBLK):
        pre_burst()
        for cp in wq_cp[b * PB:(b + 1) * PB]:
            cp.wait()
        issue(PB)
        lhs = jnp.concatenate([aq[:, s * SW + b * BW:s * SW + (b + 1) * BW] for s in range(NS)], axis=-1)
        for g in range(NG):
            qg[g] = jnp.dot(lhs, wblock(wq_v, b, g), preferred_element_type=_F32) + qg[g]
    qg = [v.astype(_BF16) for v in qg]

    scale = D ** -0.5
    tm = [[None] * NBLK for _ in range(NG)]
    for b in range(NBLK):
        pre_burst()
        for cp in wuk_cp[b * PB:(b + 1) * PB]:
            cp.wait()
        issue(PB)
        for g in range(NG):
            t = lax.dot_general(qg[g], wblock(wuk_v, b, g), _NT, preferred_element_type=_F32)
            tm[g][b] = jnp.where(diag(_HG, NS * BW), t * scale, 0.0).astype(_BF16)
    issue(len(queue))
    tn = [jnp.concatenate([tm[g][b][:, s * BW:(s + 1) * BW] for s in range(NS) for b in range(NBLK)], axis=-1)
          for g in range(NG)]
    st = jnp.concatenate([tn[g][:, a * EW:(a + 1) * EW] for a in range(C // 128) for g in range(NG)], axis=0)
    ql = lax.dot_general(st, e_v[...], _NT, preferred_element_type=_F32).astype(_BF16)
    q_lat = jnp.concatenate([ql[a * H:(a + 1) * H] for a in range(C // 128)], axis=-1)

    def make_step(pin_fn):
        def step(i, carry):
            m_old, l_old, acc, t = carry
            t = wuv_burst(sum(pre_bursts) + i * BV, BV, spin_loop, t)
            ckv_copy(i).wait()
            slot = [0]

            def pin():
                pin_fn(i, slot[0])
                slot[0] += 1

            def keys(u0, n):
                ub = 128 // RUN
                return arena[pl.ds(i * NB + u0 * ub, n * ub)].reshape(n * 128, C)

            pin()
            ss, u0 = [], 0
            for n in qk_split:
                ss.append(lax.dot_general(q_lat, keys(u0, n), _NT, preferred_element_type=_F32))
                pin()
                u0 += n
            s = jnp.concatenate(ss, axis=-1)
            m_new = jnp.maximum(m_old, jnp.max(s, axis=-1, keepdims=True))
            alpha = jnp.exp(m_old - m_new)
            p = jnp.exp(s - m_new)
            l_new = alpha * l_old + jnp.sum(p, axis=-1, keepdims=True)
            p = p.astype(_BF16)
            acc = alpha * acc
            u0 = 0
            for n in pv_split:
                acc = acc + jnp.dot(p[:, u0 * 128:(u0 + n) * 128], keys(u0, n), preferred_element_type=_F32)
                pin()
                u0 += n
            return m_new, l_new, acc, t
        return step

    carry = (jnp.full((H, 1), -jnp.inf, _F32), jnp.zeros((H, 1), _F32), jnp.zeros((H, C), _F32), pre[2])
    carry = lax.fori_loop(0, n_a, make_step(ffn_pin), carry)

    for cp in wo_cp:
        cp.start(priority=_LO)
    for src, base, sem in ((w1_hbm, B1, sem_w1), (w2_hbm, B2, sem_w2)):
        pltpu.make_async_copy(src.at[pl.ds(0, ffn_hi)], arena.at[pl.ds(base, ffn_hi)], sem).wait()
    for cp in ffn_cp:
        cp.wait()
    xn8 = jnp.broadcast_to(xn, (8, M))
    w1 = arena[B1:B1 + FB].reshape(FB * RUN, M)
    h1 = _silu(lax.dot_general(xn8, w1, _NT, preferred_element_type=_F32)).astype(_BF16)
    w2 = arena[B2:B2 + FB].reshape(FB * RUN, M)
    g_gate = _silu(jnp.dot(h1, w2, preferred_element_type=_F32))[0:1]

    _, l_fin, acc, t = lax.fori_loop(n_a, nck, make_step(wo_pin), carry)

    post = [0, n_b * npin, t]

    def post_burst():
        n = post_bursts[post[0]] if post[0] < len(post_bursts) else 0
        if n:
            k0 = post[1]

            def body(u, t):
                wo_inj(k0 + u, sem_wo)
                return spin(spin_post, t)
            post[2] = lax.fori_loop(0, n, body, post[2])
        post[0] += 1
        post[1] += n

    post_burst()
    ctx_lat = (acc / l_fin).astype(_BF16)
    av = expand(ctx_lat)
    post_burst()
    pltpu.make_async_copy(wuv_hbm, wuv_v, sem_wuv).wait()
    cg = []
    for g in range(NG):
        cg.append(jnp.dot(av[g * _HG:(g + 1) * _HG], wuv_v[:, g].reshape(C * _HG, D), preferred_element_type=_F32))
        post_burst()
    ctx = jnp.concatenate(cg, axis=0).astype(_BF16).astype(_F32)

    row8 = lax.broadcasted_iota(jnp.int32, (8, D), 0)
    lhs = jnp.concatenate(
        [jnp.where(row8 == (h % 8), ctx[(h // 8) * 8:(h // 8) * 8 + 8, :], 0.0)
         for h in range(H)], axis=-1).astype(_BF16)

    def wo_dot(lo, rows):
        return jnp.dot(lhs[:, lo:lo + rows], wo_rows_val(lo, rows), preferred_element_type=_F32)

    eye = (lax.broadcasted_iota(jnp.int32, (D, D), 0)
           == lax.broadcasted_iota(jnp.int32, (D, D), 1))
    junk[0] = post[2]
    pltpu.make_async_copy(wo_slice(wo_hbm, 0, 0, wo_lo0), wo_slice(arena, BO, 0, wo_lo0), sem_wo).wait()
    wo_cp[0].wait()
    last_col = jnp.concatenate(
        [jnp.dot(jnp.where(eye, jnp.broadcast_to(ctx[h:h + 1, :], (D, D)), 0.0).astype(_BF16),
                 jnp.ones((D, 128), _BF16), preferred_element_type=_F32)
         for h in range(H - sum(wo_vpu_rows) // D, H)], axis=0)
    lo = wo_lo0 + wo_rows[0]
    so8 = wo_dot(0, lo)
    for k, rows in enumerate(wo_rows[1:]):
        wo_cp[k + 1].wait()
        so8 = wo_dot(lo, rows) + so8
        lo += rows
    r0 = 0
    for cp, rows in zip(wo_cp[len(wo_rows):], wo_vpu_rows):
        coef = jnp.concatenate([last_col[r0:r0 + rows, :]] * (M // 128), axis=-1)
        cp.wait()
        prod = coef * wo_rows_val(lo + r0, rows).astype(_F32)
        for r in range(0, rows, 8):
            so8 = so8 + prod[r:r + 8, :]
        r0 += rows
    s = jnp.sum(so8, axis=0, keepdims=True)

    o_ref[...] = (x + s * g_gate).astype(o_ref.dtype)


def _kernel(*refs, n_sems, **kw):
    pl.run_scoped(lambda sems: _body(*refs, sems, **kw),
                  pltpu.SemaphoreType.DMA((n_sems,)))


def _forward(A_x, A_c_kv, A_w_q, A_w_uk, A_w_uv, A_w_o, B_w1, B_w2, *,
             TK=2048, n_a=8, ffn_split=0, wo_piece=16, w_passes=16, w_mr=4,
             pre_bursts=(8, 9, 9, 9, 9, 9, 9, 9, 9), spin_pre=14, spin_loop=16,
             qk_split=(3, 3, 3, 3, 2, 2), pv_split=(5, 5, 6), post_bursts=(), spin_post=12,
             wo_mxu_rows=(1024, 512), wo_vpu_rows=(256, 128, 64, 32, 16, 16)):
    B, SQ, M = A_x.shape
    _, SK, C = A_c_kv.shape
    _, H, D = A_w_q.shape
    F = B_w1.shape[1]
    RUN = 32
    NG = H // _HG
    wview = (M // (w_passes * w_mr), w_passes, w_mr, NG, _HG, D)
    n_sems = SK // TK + 5 + 1 + 2 * w_passes + 2 + 1 + len(wo_mxu_rows) + len(wo_vpu_rows)
    dt = A_x.dtype
    kernel = functools.partial(
        _kernel, n_sems=n_sems, H=H, D=D, M=M, C=C, TK=TK, n_a=n_a, ffn_split=ffn_split, wo_piece=wo_piece,
        wo_mxu_rows=wo_mxu_rows, wo_vpu_rows=wo_vpu_rows, pre_bursts=pre_bursts,
        spin_pre=spin_pre, spin_loop=spin_loop, qk_split=qk_split, pv_split=pv_split,
        post_bursts=post_bursts, spin_post=spin_post, eps=1e-5)
    any_spec = pl.BlockSpec(memory_space=pl.ANY)
    out = pl.pallas_call(
        kernel,
        in_specs=[any_spec] * 8,
        out_specs=pl.BlockSpec(memory_space=pltpu.VMEM),
        out_shape=jax.ShapeDtypeStruct((1, M), dt),
        scratch_shapes=[
            pltpu.VMEM((1, M), dt),
            pltpu.VMEM(((SK + 2 * F + H * D) // RUN, RUN, C), dt),
            pltpu.VMEM(wview, dt),
            pltpu.VMEM(wview, dt),
            pltpu.VMEM((C, NG, _HG, D), dt),
            pltpu.VMEM((128, 128 * _HG), _BF16),
            pltpu.SMEM((1,), jnp.int32),
        ],
        compiler_params=pltpu.CompilerParams(vmem_limit_bytes=100 * 1024 * 1024),
    )(
        A_x.reshape(1, M),
        A_c_kv.reshape(TK // RUN, SK // TK, RUN, C),
        A_w_q.reshape(wview),
        A_w_uk.reshape(wview),
        A_w_uv.reshape(C, NG, _HG, D),
        A_w_o.reshape(H * D // RUN, RUN, M),
        B_w1.T.reshape(F // RUN, RUN, M),
        B_w2.reshape(F // RUN, RUN, M),
    )
    return out.reshape(B, SQ, M)


@jax.jit
def pallas_recurrent_scan__compressed_kv_cla__dense_activation_silu__decode_kernel(
    A_x, A_c_kv, A_w_q, A_w_uk, A_w_uv, A_w_o, B_x, B_w1, B_w2):
    return _forward(A_x, A_c_kv, A_w_q, A_w_uk, A_w_uv, A_w_o, B_w1, B_w2)
```

```python
import functools

import jax
import jax.numpy as jnp
from jax import lax
import jax.experimental.pallas as pl
import jax.experimental.pallas.tpu as pltpu

_F32 = jnp.float32
_BF16 = jnp.bfloat16
_NT = (((1,), (1,)), ((), ()))
_LO = 1
_HG = 16
_RUN = 16
_HW = 256


def _silu(v):
    return v / (1.0 + jnp.exp(-v))


def _halves(v):
    v = v.reshape(-1, 2, 8, _HW)
    return [v[:, e].reshape(-1, _HW) for e in range(2)]


def _dot_nt(a, kh):
    return (lax.dot_general(a[:, :_HW], kh[0], _NT, preferred_element_type=_F32)
            + lax.dot_general(a[:, _HW:], kh[1], _NT, preferred_element_type=_F32))


def _dot_nn(a, kh):
    return jnp.concatenate([jnp.dot(a, k, preferred_element_type=_F32) for k in kh], axis=-1)


def _body(x_hbm, ckv_hbm, wq_hbm, wuk_hbm, wuv_hbm, wo_hbm, w1_hbm, w2_hbm,
          o_ref,
          x_v, arena, wq_v, wuk_v, wuv_v, e_v, junk, sems,
          *, H, D, M, C, lead, n_a, wo_mxu_rows, wo_vpu_rows, pre_bursts, spin_pre, spin_loop,
          qk_split, pv_split, eps):
    NSC, UC = ckv_hbm.shape[:2]
    nck = UC // _RUN
    NS, UW = wq_hbm.shape[:2]
    NG = H // _HG
    NBLK = 4
    UB = UW // NBLK
    BW = UB // NG * _HG
    SW = BW * NBLK
    EW = 128 * _HG
    FU = w1_hbm.shape[0]
    FB = -(-FU // _RUN)
    B1 = (nck + 1) * NSC
    B2 = B1 + FB
    BO = B2 + FB
    n_b = nck - n_a
    rest = _RUN - lead

    n_sem = [nck - 1]

    def new_sem():
        n_sem[0] += 1
        return sems.at[n_sem[0] - 1]

    def pass_copy(p):
        return pltpu.make_async_copy(ckv_hbm.at[:, pl.ds(lead + p * _RUN, _RUN)],
                                     arena.at[pl.ds((p + 1) * NSC, NSC)], sems.at[p])

    ckv_first = pltpu.make_async_copy(ckv_hbm.at[:, pl.ds(0, lead)],
                                      arena.at[pl.ds(0, NSC), pl.ds(rest, lead)], new_sem())
    ckv_last = pltpu.make_async_copy(ckv_hbm.at[:, pl.ds(UC - rest, rest)],
                                     arena.at[pl.ds(nck * NSC, NSC), pl.ds(0, rest)], new_sem())
    sem_w1, sem_w2, sem_wuv, sem_wo = (new_sem() for _ in range(4))

    def spin(n, t):
        return lax.fori_loop(0, n, lambda i, t: t * 5 + i, t)

    PV = 2
    NV = C // PV
    BV = (NV - sum(pre_bursts)) // (nck - 1)
    assert sum(pre_bursts) + BV * (nck - 1) == NV

    def wuv_burst(k0, n, nspin, t):
        def body(u, t):
            o = (k0 + u) * PV
            pltpu.make_async_copy(wuv_hbm.at[pl.ds(o, PV)], wuv_v.at[pl.ds(o, PV)], sem_wuv).start()
            return spin(nspin, t)
        return lax.fori_loop(0, n, body, t)

    npin = 1 + len(qk_split) + len(pv_split)
    HB = _RUN // 2
    ffn_hi = npin // 2 * n_a // 2
    assert npin % 2 == 0 and (npin // 2 * n_a) % 2 == 0 and ffn_hi * _RUN <= FU

    def ffn_pin(i, slot):
        src, base, sem = ((w1_hbm, B1, sem_w1), (w2_hbm, B2, sem_w2))[slot % 2]
        k = i * (npin // 2) + slot // 2
        pltpu.make_async_copy(src.at[pl.ds(k * HB, HB)],
                              arena.at[base + k // 2, pl.ds((k % 2) * HB, HB)], sem).start()

    QB = _RUN // 4

    def wo_pin(i, slot):
        k = (i - n_a) * npin + slot
        r = pl.ds((k % 4) * QB, QB)
        pltpu.make_async_copy(wo_hbm.at[k // 4, r], arena.at[BO + k // 4, r], sem_wo).start()

    RB = _RUN * 4
    wo_hi = n_b * npin * QB * 4
    assert wo_hi % RB == 0

    def wo_slice(ref, base, lo, rows):
        if lo % RB == 0 and rows % RB == 0:
            return ref.at[pl.ds(base + lo // RB, rows // RB)]
        assert lo // RB == (lo + rows - 1) // RB
        return ref.at[base + lo // RB, pl.ds(lo % RB // 4, rows // 4)]

    def weight_copies(src, dst):
        cuts = [0] + list(range(lead, UW, _RUN)) + [UW]
        return [pltpu.make_async_copy(src.at[:, pl.ds(a, b - a)], dst.at[:, pl.ds(a, b - a)], new_sem())
                for a, b in zip(cuts[:-1], cuts[1:])], cuts[1:]

    x_cp = pltpu.make_async_copy(x_hbm, x_v, new_sem())
    wq_cp, w_ends = weight_copies(wq_hbm, wq_v)
    wuk_cp, _ = weight_copies(wuk_hbm, wuk_v)
    ffn_cp = []
    for src, base in ((w1_hbm, B1), (w2_hbm, B2)):
        for b in range(ffn_hi, FB):
            n = min(_RUN, FU - b * _RUN)
            ffn_cp.append(pltpu.make_async_copy(src.at[pl.ds(b * _RUN, n)],
                                                arena.at[base + b, pl.ds(0, n)], new_sem()))
    wo_rows = (H * D - wo_hi - sum(wo_mxu_rows) - sum(wo_vpu_rows),) + tuple(wo_mxu_rows)
    assert wo_rows[0] > 0
    wo_cp = []
    lo = wo_hi
    for rows in wo_rows + tuple(wo_vpu_rows):
        wo_cp.append(pltpu.make_async_copy(wo_slice(wo_hbm, 0, lo, rows),
                                           wo_slice(arena, BO, lo, rows), new_sem()))
        lo += rows

    queue = ([x_cp] + wq_cp + wuk_cp + ffn_cp + [ckv_first]
             + [pass_copy(p) for p in range(nck - 1)] + [ckv_last])
    issued = [0]

    def issue(n):
        for cp in queue[issued[0]:issued[0] + n]:
            cp.start(priority=_LO)
        issued[0] = min(len(queue), issued[0] + n)

    issue(24)

    pre = [0, 0, jnp.int32(1)]

    def pre_burst():
        n = pre_bursts[pre[0]]
        if n:
            pre[2] = wuv_burst(pre[1], n, spin_pre, pre[2])
        pre[0] += 1
        pre[1] += n

    ei = lax.broadcasted_iota(jnp.int32, (128, EW), 0)
    ej = lax.broadcasted_iota(jnp.int32, (128, EW), 1)
    e_v[...] = jnp.where(ej // _HG == ei, 1.0, 0.0).astype(_BF16)

    def diag(rows, cols):
        di = lax.broadcasted_iota(jnp.int32, (rows, cols), 0)
        dj = lax.broadcasted_iota(jnp.int32, (rows, cols), 1)
        return (dj % _HG) == (di % _HG)

    def expand(v):
        R, K = v.shape
        st = jnp.concatenate([v[:, a * 128:(a + 1) * 128] for a in range(K // 128)], axis=0)
        ex = jnp.dot(st, e_v[...], preferred_element_type=_F32)
        ex = jnp.where(diag(st.shape[0], EW), ex, 0.0).astype(_BF16)
        return jnp.concatenate([ex[a * R:(a + 1) * R] for a in range(K // 128)], axis=-1)

    pre_burst()
    x_cp.wait()
    x = x_v[...].astype(_F32)
    mu = jnp.mean(x, axis=-1, keepdims=True)
    xc = x - mu
    var = jnp.mean(xc * xc, axis=-1, keepdims=True)
    xn = (xc / jnp.sqrt(var + eps)).astype(_BF16)
    aq = expand(jnp.broadcast_to(xn, (_HG, M)))

    def wblock(ref, b):
        v = ref[:, b * UB:(b + 1) * UB].reshape(-1, NG, _HG, D)
        return [v[:, g].reshape(NS * BW, D) for g in range(NG)]

    def wait_block(cps, b, done):
        while done < len(cps) and (done == 0 or w_ends[done - 1] < (b + 1) * UB):
            cps[done].wait()
            issue(1)
            done += 1
        return done

    qg = [jnp.zeros((_HG, D), _F32) for _ in range(NG)]
    done = 0
    for b in range(NBLK):
        pre_burst()
        done = wait_block(wq_cp, b, done)
        lhs = jnp.concatenate([aq[:, s * SW + b * BW:s * SW + (b + 1) * BW] for s in range(NS)], axis=-1)
        for g, w in enumerate(wblock(wq_v, b)):
            qg[g] = jnp.dot(lhs, w, preferred_element_type=_F32) + qg[g]
    qg = [v.astype(_BF16) for v in qg]

    scale = D ** -0.5
    tm = [[None] * NBLK for _ in range(NG)]
    done = 0
    for b in range(NBLK):
        pre_burst()
        done = wait_block(wuk_cp, b, done)
        for g, w in enumerate(wblock(wuk_v, b)):
            t = lax.dot_general(qg[g], w, _NT, preferred_element_type=_F32)
            tm[g][b] = jnp.where(diag(_HG, NS * BW), t * scale, 0.0).astype(_BF16)
    issue(len(queue))
    tn = [jnp.concatenate([tm[g][b][:, s * BW:(s + 1) * BW] for s in range(NS) for b in range(NBLK)], axis=-1)
          for g in range(NG)]
    st = jnp.concatenate([tn[g][:, a * EW:(a + 1) * EW] for a in range(C // 128) for g in range(NG)], axis=0)
    ql = lax.dot_general(st, e_v[...], _NT, preferred_element_type=_F32).astype(_BF16)
    q_lat = jnp.concatenate([ql[a * H:(a + 1) * H] for a in range(C // 128)], axis=-1)
    pre_burst()
    ckv_first.wait()

    SK128 = 128 // (_RUN * 4)

    def make_step(pin_fn, has_last):
        def step(i, carry):
            m_old, l_old, acc, t = carry
            nb = jnp.where(i == nck - 1, 0, BV) if has_last else BV
            t = wuv_burst(sum(pre_bursts) + i * BV, nb, spin_loop, t)
            if has_last:
                pl.when(i < nck - 1)(lambda: pass_copy(i).wait())
                pl.when(i == nck - 1)(ckv_last.wait)
            else:
                pass_copy(i).wait()
            slot = [0]

            def pin():
                pin_fn(i, slot[0])
                slot[0] += 1

            def keys(u0, n):
                a = arena[pl.ds(i * NSC + u0 * SK128, n * SK128), rest:_RUN]
                b = arena[pl.ds((i + 1) * NSC + u0 * SK128, n * SK128), 0:rest]
                return _halves(jnp.concatenate([a, b], axis=1))

            pin()
            ss, u0 = [], 0
            for n in qk_split:
                ss.append(_dot_nt(q_lat, keys(u0, n)))
                pin()
                u0 += n
            s = jnp.concatenate(ss, axis=-1)
            m_new = jnp.maximum(m_old, jnp.max(s, axis=-1, keepdims=True))
            alpha = jnp.exp(m_old - m_new)
            p = jnp.exp(s - m_new)
            l_new = alpha * l_old + jnp.sum(p, axis=-1, keepdims=True)
            p = p.astype(_BF16)
            acc = alpha * acc
            u0 = 0
            for n in pv_split:
                acc = _dot_nn(p[:, u0 * 128:(u0 + n) * 128], keys(u0, n)) + acc
                pin()
                u0 += n
            return m_new, l_new, acc, t
        return step

    carry = (jnp.full((H, 1), -jnp.inf, _F32), jnp.zeros((H, 1), _F32), jnp.zeros((H, C), _F32), pre[2])
    carry = lax.fori_loop(0, n_a, make_step(ffn_pin, False), carry)

    for cp in wo_cp:
        cp.start(priority=_LO)
    for base, sem in ((B1, sem_w1), (B2, sem_w2)):
        dst = arena.at[pl.ds(base, ffn_hi)]
        pltpu.make_async_copy(dst, dst, sem).wait()
    for cp in ffn_cp:
        cp.wait()

    def ffn_weight(base):
        full, part = FU // _RUN, FU % _RUN
        v = arena[base:base + full].reshape(full * _RUN, 8, _HW)
        if part:
            v = jnp.concatenate([v, arena[base + full, 0:part]], axis=0)
        return _halves(v)

    xn8 = jnp.broadcast_to(xn, (8, M))
    h1 = _silu(_dot_nt(xn8, ffn_weight(B1))).astype(_BF16)
    g_gate = _silu(_dot_nn(h1, ffn_weight(B2)))[0:1]

    _, l_fin, acc, t = lax.fori_loop(n_a, nck, make_step(wo_pin, True), carry)
    junk[0] = t

    ctx_lat = (acc / l_fin).astype(_BF16)
    av = expand(ctx_lat)
    pltpu.make_async_copy(wuv_v, wuv_v, sem_wuv).wait()
    ctx = jnp.concatenate(
        [jnp.dot(av[g * _HG:(g + 1) * _HG], wuv_v[:, g].reshape(C * _HG, D), preferred_element_type=_F32)
         for g in range(NG)], axis=0).astype(_BF16).astype(_F32)

    row8 = lax.broadcasted_iota(jnp.int32, (8, D), 0)
    lhs = jnp.concatenate(
        [jnp.where(row8 == (h % 8), ctx[(h // 8) * 8:(h // 8) * 8 + 8, :], 0.0)
         for h in range(H)], axis=-1).astype(_BF16)

    def wo_dot(lo, rows):
        return _dot_nn(lhs[:, lo:lo + rows], _halves(wo_slice(arena, BO, lo, rows)[...]))

    eye = (lax.broadcasted_iota(jnp.int32, (D, D), 0)
           == lax.broadcasted_iota(jnp.int32, (D, D), 1))
    dst = wo_slice(arena, BO, 0, wo_hi)
    pltpu.make_async_copy(dst, dst, sem_wo).wait()
    wo_cp[0].wait()
    last_col = jnp.concatenate(
        [jnp.dot(jnp.where(eye, jnp.broadcast_to(ctx[h:h + 1, :], (D, D)), 0.0).astype(_BF16),
                 jnp.ones((D, 128), _BF16), preferred_element_type=_F32)
         for h in range(H - sum(wo_vpu_rows) // D, H)], axis=0)
    lo = wo_hi + wo_rows[0]
    so8 = wo_dot(0, lo)
    for k, rows in enumerate(wo_rows[1:]):
        wo_cp[k + 1].wait()
        so8 = wo_dot(lo, rows) + so8
        lo += rows
    r0 = 0
    for cp, rows in zip(wo_cp[len(wo_rows):], wo_vpu_rows):
        coef = jnp.concatenate([last_col[r0:r0 + rows, :]] * (M // 128), axis=-1)
        cp.wait()
        w = jnp.concatenate(_halves(wo_slice(arena, BO, lo + r0, rows)[...].astype(_F32)), axis=-1)
        prod = coef * w
        for r in range(0, rows, 8):
            so8 = so8 + prod[r:r + 8, :]
        r0 += rows
    s = jnp.sum(so8, axis=0, keepdims=True)

    o_ref[...] = (x + s * g_gate).astype(o_ref.dtype)


def _kernel(*refs, n_sems, **kw):
    pl.run_scoped(lambda sems: _body(*refs, sems, **kw),
                  pltpu.SemaphoreType.DMA((n_sems,)))


def _units(a):
    rows = a.shape[0]
    return a.reshape(rows // 8, 8, 2, _HW).transpose(0, 2, 1, 3).reshape(rows // 4, 8, _HW)


def _forward(A_x, A_c_kv, A_w_q, A_w_uk, A_w_uv, A_w_o, B_w1, B_w2, *,
             nck=16, lead=7, n_a=8, w_strides=8,
             pre_bursts=(8, 12, 9, 9, 5, 12, 9, 9, 5, 13), spin_pre=14, spin_loop=16,
             qk_split=(3, 3, 3, 3, 2, 2), pv_split=(5, 5, 6),
             wo_mxu_rows=(1024, 512), wo_vpu_rows=(256, 128, 64, 32, 16, 16)):
    B, SQ, M = A_x.shape
    _, SK, C = A_c_kv.shape
    _, H, D = A_w_q.shape
    F = B_w1.shape[1]
    NG = H // _HG
    nsc = SK // 4 // (nck * _RUN)
    wview = (w_strides, M * NG // w_strides, _HG, D)
    fb = -(-(F // 4) // _RUN)
    n_sems = 80
    dt = A_x.dtype
    kernel = functools.partial(
        _kernel, n_sems=n_sems, H=H, D=D, M=M, C=C, lead=lead, n_a=n_a,
        wo_mxu_rows=wo_mxu_rows, wo_vpu_rows=wo_vpu_rows, pre_bursts=pre_bursts,
        spin_pre=spin_pre, spin_loop=spin_loop, qk_split=qk_split, pv_split=pv_split, eps=1e-5)
    any_spec = pl.BlockSpec(memory_space=pl.ANY)
    out = pl.pallas_call(
        kernel,
        in_specs=[any_spec] * 8,
        out_specs=pl.BlockSpec(memory_space=pltpu.VMEM),
        out_shape=jax.ShapeDtypeStruct((1, M), dt),
        scratch_shapes=[
            pltpu.VMEM((1, M), dt),
            pltpu.VMEM(((nck + 1) * nsc + 2 * fb + H * D // 4 // _RUN, _RUN, 8, _HW), dt),
            pltpu.VMEM(wview, dt),
            pltpu.VMEM(wview, dt),
            pltpu.VMEM((C, NG, _HG, D), dt),
            pltpu.VMEM((128, 128 * _HG), _BF16),
            pltpu.SMEM((1,), jnp.int32),
        ],
        compiler_params=pltpu.CompilerParams(vmem_limit_bytes=100 * 1024 * 1024),
    )(
        A_x.reshape(1, M),
        _units(A_c_kv.reshape(SK, C)).reshape(nsc, nck * _RUN, 8, _HW),
        A_w_q.reshape(wview),
        A_w_uk.reshape(wview),
        A_w_uv.reshape(C, NG, _HG, D),
        _units(A_w_o.reshape(H * D, M)).reshape(H * D // 4 // _RUN, _RUN, 8, _HW),
        _units(B_w1.T),
        _units(B_w2),
    )
    return out.reshape(B, SQ, M)


@jax.jit
def pallas_recurrent_scan__compressed_kv_cla__dense_activation_silu__decode_kernel(
    A_x, A_c_kv, A_w_q, A_w_uk, A_w_uv, A_w_o, B_x, B_w1, B_w2):
    return _forward(A_x, A_c_kv, A_w_q, A_w_uk, A_w_uv, A_w_o, B_w1, B_w2)
```

```python
import functools

import jax
import jax.numpy as jnp
from jax import lax
import jax.experimental.pallas as pl
import jax.experimental.pallas.tpu as pltpu

_F32 = jnp.float32
_BF16 = jnp.bfloat16
_NT = (((1,), (1,)), ((), ()))
_LO = 1
_HG = 16
_RUN = 16
_HW = 256


def _silu(v):
    return v / (1.0 + jnp.exp(-v))


def _halves(v):
    v = v.reshape(-1, 2, 8, _HW)
    return [v[:, e].reshape(-1, _HW) for e in range(2)]


def _dot_nt(a, kh):
    return (lax.dot_general(a[:, :_HW], kh[0], _NT, preferred_element_type=_F32)
            + lax.dot_general(a[:, _HW:], kh[1], _NT, preferred_element_type=_F32))


def _dot_nn(a, kh):
    return jnp.concatenate([jnp.dot(a, k, preferred_element_type=_F32) for k in kh], axis=-1)


def _body(x_hbm, ckv_hbm, wq_hbm, wuk_hbm, wuv_hbm, wo_hbm, w1_hbm, w2_hbm,
          o_ref,
          x_v, arena, wq_v, wuk_v, wuv_v, e_v, sink, sems,
          *, H, D, M, C, lead, n_a, wo_mxu_rows, wo_vpu_rows, pre_bursts, spin_pre, spin_loop,
          qk_split, pv_split, eps):
    NSC, UC = ckv_hbm.shape[:2]
    nck = UC // _RUN
    NS, UW = wq_hbm.shape[:2]
    NG = H // _HG
    NBLK = 4
    UB = UW // NBLK
    BW = UB // NG * _HG
    SW = BW * NBLK
    EW = 128 * _HG
    FU = w1_hbm.shape[0]
    FB = -(-FU // _RUN)
    B1 = (nck + 1) * NSC
    B2 = B1 + FB
    BO = B2 + FB
    n_b = nck - n_a
    rest = _RUN - lead

    n_sem = [nck - 1]

    def new_sem():
        n_sem[0] += 1
        return sems.at[n_sem[0] - 1]

    def pass_copy(p):
        return pltpu.make_async_copy(ckv_hbm.at[:, pl.ds(lead + p * _RUN, _RUN)],
                                     arena.at[pl.ds((p + 1) * NSC, NSC)], sems.at[p])

    ckv_first = pltpu.make_async_copy(ckv_hbm.at[:, pl.ds(0, lead)],
                                      arena.at[pl.ds(0, NSC), pl.ds(rest, lead)], new_sem())
    ckv_last = pltpu.make_async_copy(ckv_hbm.at[:, pl.ds(UC - rest, rest)],
                                     arena.at[pl.ds(nck * NSC, NSC), pl.ds(0, rest)], new_sem())

    sem_w1, sem_w2, sem_wuv, sem_wo = (new_sem() for _ in range(4))

    def wait_total(dst, sem):
        pltpu.make_async_copy(dst, dst, sem).wait()

    PV = 2
    NV = C // PV
    BV = (NV - sum(pre_bursts)) // (nck - 1)
    assert sum(pre_bursts) + BV * (nck - 1) == NV

    def wuv_burst(k0, n, nspin, t):
        def body(u, t):
            o = (k0 + u) * PV
            pltpu.make_async_copy(wuv_hbm.at[pl.ds(o, PV)], wuv_v.at[pl.ds(o, PV)], sem_wuv).start()
            return lax.fori_loop(0, nspin, lambda i, t: t * 5 + i, t)
        return lax.fori_loop(0, n, body, t)

    npin = 1 + len(qk_split) + len(pv_split)
    HB = _RUN // 2
    ffn_hi = npin // 2 * n_a // 2
    assert npin % 2 == 0 and (npin // 2 * n_a) % 2 == 0 and ffn_hi * _RUN <= FU

    def ffn_pin(i, slot):
        src, base, sem = ((w1_hbm, B1, sem_w1), (w2_hbm, B2, sem_w2))[slot % 2]
        k = i * (npin // 2) + slot // 2
        pltpu.make_async_copy(src.at[pl.ds(k * HB, HB)],
                              arena.at[base + k // 2, pl.ds((k % 2) * HB, HB)], sem).start()

    QB = _RUN // 4

    def wo_pin(i, slot):
        k = (i - n_a) * npin + slot
        r = pl.ds((k % 4) * QB, QB)
        pltpu.make_async_copy(wo_hbm.at[k // 4, r], arena.at[BO + k // 4, r], sem_wo).start()

    RB = _RUN * 4
    wo_hi = n_b * npin * QB * 4
    assert wo_hi % RB == 0

    def wo_slice(ref, base, lo, rows):
        if lo % RB == 0 and rows % RB == 0:
            return ref.at[pl.ds(base + lo // RB, rows // RB)]
        assert lo // RB == (lo + rows - 1) // RB
        return ref.at[base + lo // RB, pl.ds(lo % RB // 4, rows // 4)]

    def weight_copies(src, dst):
        cuts = [0] + list(range(lead, UW, _RUN)) + [UW]
        return [pltpu.make_async_copy(src.at[:, pl.ds(a, b - a)], dst.at[:, pl.ds(a, b - a)], new_sem())
                for a, b in zip(cuts[:-1], cuts[1:])], cuts[1:]

    x_cp = pltpu.make_async_copy(x_hbm, x_v, new_sem())
    wq_cp, w_ends = weight_copies(wq_hbm, wq_v)
    wuk_cp, _ = weight_copies(wuk_hbm, wuk_v)
    ffn_cp = []
    for src, base in ((w1_hbm, B1), (w2_hbm, B2)):
        for b in range(ffn_hi, FB):
            n = min(_RUN, FU - b * _RUN)
            ffn_cp.append(pltpu.make_async_copy(src.at[pl.ds(b * _RUN, n)],
                                                arena.at[base + b, pl.ds(0, n)], new_sem()))
    wo_rows = (H * D - wo_hi - sum(wo_mxu_rows) - sum(wo_vpu_rows),) + tuple(wo_mxu_rows)
    assert wo_rows[0] > 0 and sum(wo_vpu_rows) % D == 0
    wo_cp = []
    lo = wo_hi
    for rows in wo_rows + tuple(wo_vpu_rows):
        wo_cp.append(pltpu.make_async_copy(wo_slice(wo_hbm, 0, lo, rows),
                                           wo_slice(arena, BO, lo, rows), new_sem()))
        lo += rows
    assert n_sem[0] <= sems.shape[0]

    queue = ([x_cp] + wq_cp + wuk_cp + ffn_cp + [ckv_first]
             + [pass_copy(p) for p in range(nck - 1)] + [ckv_last])
    issued = [0]

    def issue(n):
        for cp in queue[issued[0]:issued[0] + n]:
            cp.start(priority=_LO)
        issued[0] = min(len(queue), issued[0] + n)

    issue(24)

    pre = [0, 0, jnp.int32(1)]

    def pre_burst():
        n = pre_bursts[pre[0]]
        if n:
            pre[2] = wuv_burst(pre[1], n, spin_pre, pre[2])
        pre[0] += 1
        pre[1] += n

    ei = lax.broadcasted_iota(jnp.int32, (128, EW), 0)
    ej = lax.broadcasted_iota(jnp.int32, (128, EW), 1)
    e_v[...] = jnp.where(ej // _HG == ei, 1.0, 0.0).astype(_BF16)

    def diag(rows, cols):
        di = lax.broadcasted_iota(jnp.int32, (rows, cols), 0)
        dj = lax.broadcasted_iota(jnp.int32, (rows, cols), 1)
        return (dj % _HG) == (di % _HG)

    def expand(v):
        R, K = v.shape
        st = jnp.concatenate([v[:, a * 128:(a + 1) * 128] for a in range(K // 128)], axis=0)
        ex = jnp.dot(st, e_v[...], preferred_element_type=_F32)
        ex = jnp.where(diag(st.shape[0], EW), ex, 0.0).astype(_BF16)
        return jnp.concatenate([ex[a * R:(a + 1) * R] for a in range(K // 128)], axis=-1)

    pre_burst()
    x_cp.wait()
    x = x_v[...].astype(_F32)
    mu = jnp.mean(x, axis=-1, keepdims=True)
    xc = x - mu
    var = jnp.mean(xc * xc, axis=-1, keepdims=True)
    xn = (xc / jnp.sqrt(var + eps)).astype(_BF16)
    aq = expand(jnp.broadcast_to(xn, (_HG, M)))

    def wblock(ref, b):
        v = ref[:, b * UB:(b + 1) * UB].reshape(-1, NG, _HG, D)
        return [v[:, g].reshape(NS * BW, D) for g in range(NG)]

    def wait_block(cps, b, done):
        while done < len(cps) and (done == 0 or w_ends[done - 1] < (b + 1) * UB):
            cps[done].wait()
            issue(1)
            done += 1
        return done

    qg = [jnp.zeros((_HG, D), _F32) for _ in range(NG)]
    done = 0
    for b in range(NBLK):
        pre_burst()
        done = wait_block(wq_cp, b, done)
        lhs = jnp.concatenate([aq[:, s * SW + b * BW:s * SW + (b + 1) * BW] for s in range(NS)], axis=-1)
        for g, w in enumerate(wblock(wq_v, b)):
            qg[g] = jnp.dot(lhs, w, preferred_element_type=_F32) + qg[g]
    qg = [v.astype(_BF16) for v in qg]

    scale = D ** -0.5
    tm = [[None] * NBLK for _ in range(NG)]
    done = 0
    for b in range(NBLK):
        pre_burst()
        done = wait_block(wuk_cp, b, done)
        for g, w in enumerate(wblock(wuk_v, b)):
            t = lax.dot_general(qg[g], w, _NT, preferred_element_type=_F32)
            tm[g][b] = jnp.where(diag(_HG, NS * BW), t * scale, 0.0).astype(_BF16)
    issue(len(queue))
    tn = [jnp.concatenate([tm[g][b][:, s * BW:(s + 1) * BW] for s in range(NS) for b in range(NBLK)], axis=-1)
          for g in range(NG)]
    st = jnp.concatenate([tn[g][:, a * EW:(a + 1) * EW] for a in range(C // 128) for g in range(NG)], axis=0)
    ql = lax.dot_general(st, e_v[...], _NT, preferred_element_type=_F32).astype(_BF16)
    q_lat = jnp.concatenate([ql[a * H:(a + 1) * H] for a in range(C // 128)], axis=-1)
    pre_burst()
    ckv_first.wait()

    SK128 = 128 // (_RUN * 4)

    def make_step(pin_fn, has_last):
        def step(i, carry):
            m_old, l_old, acc, t = carry
            nb = jnp.where(i == nck - 1, 0, BV) if has_last else BV
            t = wuv_burst(sum(pre_bursts) + i * BV, nb, spin_loop, t)
            if has_last:
                pl.when(i < nck - 1)(lambda: pass_copy(i).wait())
                pl.when(i == nck - 1)(ckv_last.wait)
            else:
                pass_copy(i).wait()
            slot = [0]

            def pin():
                pin_fn(i, slot[0])
                slot[0] += 1

            def keys(u0, n):
                a = arena[pl.ds(i * NSC + u0 * SK128, n * SK128), rest:_RUN]
                b = arena[pl.ds((i + 1) * NSC + u0 * SK128, n * SK128), 0:rest]
                return _halves(jnp.concatenate([a, b], axis=1))

            pin()
            ss, u0 = [], 0
            for n in qk_split:
                ss.append(_dot_nt(q_lat, keys(u0, n)))
                pin()
                u0 += n
            s = jnp.concatenate(ss, axis=-1)
            m_new = jnp.maximum(m_old, jnp.max(s, axis=-1, keepdims=True))
            alpha = jnp.exp(m_old - m_new)
            p = jnp.exp(s - m_new)
            l_new = alpha * l_old + jnp.sum(p, axis=-1, keepdims=True)
            p = p.astype(_BF16)
            acc = alpha * acc
            u0 = 0
            for n in pv_split:
                acc = _dot_nn(p[:, u0 * 128:(u0 + n) * 128], keys(u0, n)) + acc
                pin()
                u0 += n
            return m_new, l_new, acc, t
        return step

    assert sum(qk_split) * SK128 == NSC and sum(pv_split) * SK128 == NSC
    carry = (jnp.full((H, 1), -jnp.inf, _F32), jnp.zeros((H, 1), _F32), jnp.zeros((H, C), _F32), pre[2])
    carry = lax.fori_loop(0, n_a, make_step(ffn_pin, False), carry)

    for cp in wo_cp:
        cp.start(priority=_LO)
    wait_total(arena.at[pl.ds(B1, ffn_hi)], sem_w1)
    wait_total(arena.at[pl.ds(B2, ffn_hi)], sem_w2)
    for cp in ffn_cp:
        cp.wait()

    def ffn_weight(base):
        full, part = FU // _RUN, FU % _RUN
        v = arena[base:base + full].reshape(full * _RUN, 8, _HW)
        if part:
            v = jnp.concatenate([v, arena[base + full, 0:part]], axis=0)
        return _halves(v)

    xn8 = jnp.broadcast_to(xn, (8, M))
    h1 = _silu(_dot_nt(xn8, ffn_weight(B1))).astype(_BF16)
    gate = _silu(_dot_nn(h1, ffn_weight(B2)))[0:1]

    _, l_fin, acc, t = lax.fori_loop(n_a, nck, make_step(wo_pin, True), carry)
    sink[0] = t

    av = expand((acc / l_fin).astype(_BF16))
    wait_total(wuv_v, sem_wuv)
    ctx = jnp.concatenate(
        [jnp.dot(av[g * _HG:(g + 1) * _HG], wuv_v[:, g].reshape(C * _HG, D), preferred_element_type=_F32)
         for g in range(NG)], axis=0).astype(_BF16).astype(_F32)

    row8 = lax.broadcasted_iota(jnp.int32, (8, D), 0)
    lhs = jnp.concatenate(
        [jnp.where(row8 == (h % 8), ctx[(h // 8) * 8:(h // 8) * 8 + 8, :], 0.0)
         for h in range(H)], axis=-1).astype(_BF16)

    def wo_dot(lo, rows):
        return _dot_nn(lhs[:, lo:lo + rows], _halves(wo_slice(arena, BO, lo, rows)[...]))

    wait_total(wo_slice(arena, BO, 0, wo_hi), sem_wo)
    wo_cp[0].wait()
    eye = (lax.broadcasted_iota(jnp.int32, (D, D), 0)
           == lax.broadcasted_iota(jnp.int32, (D, D), 1))
    last_col = jnp.concatenate(
        [jnp.dot(jnp.where(eye, jnp.broadcast_to(ctx[h:h + 1, :], (D, D)), 0.0).astype(_BF16),
                 jnp.ones((D, 128), _BF16), preferred_element_type=_F32)
         for h in range(H - sum(wo_vpu_rows) // D, H)], axis=0)
    lo = wo_hi + wo_rows[0]
    so8 = wo_dot(0, lo)
    for k, rows in enumerate(wo_rows[1:]):
        wo_cp[k + 1].wait()
        so8 = wo_dot(lo, rows) + so8
        lo += rows
    r0 = 0
    for cp, rows in zip(wo_cp[len(wo_rows):], wo_vpu_rows):
        coef = jnp.concatenate([last_col[r0:r0 + rows, :]] * (M // 128), axis=-1)
        cp.wait()
        w = jnp.concatenate(_halves(wo_slice(arena, BO, lo + r0, rows)[...].astype(_F32)), axis=-1)
        prod = coef * w
        for r in range(0, rows, 8):
            so8 = so8 + prod[r:r + 8, :]
        r0 += rows
    s = jnp.sum(so8, axis=0, keepdims=True)

    o_ref[...] = (x + s * gate).astype(o_ref.dtype)


def _kernel(*refs, n_sems, **kw):
    pl.run_scoped(lambda sems: _body(*refs, sems, **kw),
                  pltpu.SemaphoreType.DMA((n_sems,)))


def _units(a):
    rows = a.shape[0]
    return a.reshape(rows // 8, 8, 2, _HW).transpose(0, 2, 1, 3).reshape(rows // 4, 8, _HW)


def _forward(A_x, A_c_kv, A_w_q, A_w_uk, A_w_uv, A_w_o, B_w1, B_w2, *,
             nck=16, lead=7, n_a=8, w_strides=8,
             pre_bursts=(9, 14, 11, 11, 6, 14, 11, 11, 6, 13), spin_pre=11, spin_loop=18,
             qk_split=(3, 3, 3, 3, 2, 2), pv_split=(5, 5, 6),
             wo_mxu_rows=(1024, 512), wo_vpu_rows=(256, 128, 64, 32, 16, 16)):
    B, SQ, M = A_x.shape
    _, SK, C = A_c_kv.shape
    _, H, D = A_w_q.shape
    F = B_w1.shape[1]
    assert B == 1 and SQ == 1 and D == 128 and H == 2 * _HG and M == 2 * _HW and C == 2 * _HW
    assert F % 32 == 0 and 0 < lead < _RUN
    NG = H // _HG
    nsc = SK // 4 // (nck * _RUN)
    wview = (w_strides, M * NG // w_strides, _HG, D)
    fb = -(-(F // 4) // _RUN)
    dt = A_x.dtype
    kernel = functools.partial(
        _kernel, n_sems=64, H=H, D=D, M=M, C=C, lead=lead, n_a=n_a,
        wo_mxu_rows=wo_mxu_rows, wo_vpu_rows=wo_vpu_rows, pre_bursts=pre_bursts,
        spin_pre=spin_pre, spin_loop=spin_loop, qk_split=qk_split, pv_split=pv_split, eps=1e-5)
    any_spec = pl.BlockSpec(memory_space=pl.ANY)
    out = pl.pallas_call(
        kernel,
        in_specs=[any_spec] * 8,
        out_specs=pl.BlockSpec(memory_space=pltpu.VMEM),
        out_shape=jax.ShapeDtypeStruct((1, M), dt),
        scratch_shapes=[
            pltpu.VMEM((1, M), dt),
            pltpu.VMEM(((nck + 1) * nsc + 2 * fb + H * D // 4 // _RUN, _RUN, 8, _HW), dt),
            pltpu.VMEM(wview, dt),
            pltpu.VMEM(wview, dt),
            pltpu.VMEM((C, NG, _HG, D), dt),
            pltpu.VMEM((128, 128 * _HG), _BF16),
            pltpu.SMEM((1,), jnp.int32),
        ],
        compiler_params=pltpu.CompilerParams(vmem_limit_bytes=100 * 1024 * 1024),
    )(
        A_x.reshape(1, M),
        _units(A_c_kv.reshape(SK, C)).reshape(nsc, nck * _RUN, 8, _HW),
        A_w_q.reshape(wview),
        A_w_uk.reshape(wview),
        A_w_uv.reshape(C, NG, _HG, D),
        _units(A_w_o.reshape(H * D, M)).reshape(H * D // 4 // _RUN, _RUN, 8, _HW),
        _units(B_w1.T),
        _units(B_w2),
    )
    return out.reshape(B, SQ, M)


@jax.jit
def pallas_recurrent_scan__compressed_kv_cla__dense_activation_silu__decode_kernel(
    A_x: jax.Array,
    A_c_kv: jax.Array,
    A_w_q: jax.Array,
    A_w_uk: jax.Array,
    A_w_uv: jax.Array,
    A_w_o: jax.Array,
    B_x: jax.Array,
    B_w1: jax.Array,
    B_w2: jax.Array,
):
    return _forward(A_x, A_c_kv, A_w_q, A_w_uk, A_w_uv, A_w_o, B_w1, B_w2)
```

```python
import functools

import jax
import jax.numpy as jnp
from jax import lax
import jax.experimental.pallas as pl
import jax.experimental.pallas.tpu as pltpu

_F32 = jnp.float32
_BF16 = jnp.bfloat16
_LO = 1
_HW = 256
_RUN = 16
_ROW = 128


def _silu(v):
    return v / (1.0 + jnp.exp(-v))


def _iota(shape, dim):
    return lax.broadcasted_iota(jnp.int32, shape, dim)


def _halves(v):
    v = v.reshape(-1, 2, 8, _HW)
    return [v[:, e].reshape(-1, _HW) for e in range(2)]


def _dot(a, b):
    return jnp.dot(a, b, preferred_element_type=_F32)


def _dot_t(a, b):
    return lax.dot_general(a, b, (((1,), (1,)), ((), ())), preferred_element_type=_F32)


def _dot_nt(a, kh):
    return _dot_t(a[:, :_HW], kh[0]) + _dot_t(a[:, _HW:], kh[1])


def _dot_nn(a, kh):
    return jnp.concatenate([_dot(a, k) for k in kh], axis=-1)


def _body(x_hbm, ckv_hbm, wq_hbm, wuk_hbm, wuv_hbm, wo_hbm, w1_hbm, w2_hbm,
          o_ref, x_v, arena, e_v, sink, sems,
          *, H, D, M, C, lead, pre_bursts, spin_pre, spin_loop, qk_split, pv_split, eps):
    NC = ckv_hbm.shape[0] // 2
    NS = wq_hbm.shape[0]
    FU = w1_hbm.shape[0]
    FR = -(-FU // _ROW)
    RQ = 2 * NC
    RK, RV, RO = RQ + NS, RQ + 2 * NS, RQ + 3 * NS
    R1 = RO + NS
    R2 = R1 + FR
    NJ = _ROW // _RUN
    NBLK = 4
    UB = _ROW // NBLK
    EW = 128 * 8
    cuts = [0] + list(range(lead, _ROW, _RUN)) + [_ROW]

    n_sem = [2 * (NJ - 1)]

    def new_sem(n=1):
        n_sem[0] += n
        return n_sem[0] - n

    def rect(src, base, s0, rows, a, b):
        return pltpu.make_async_copy(src.at[pl.ds(s0, rows), pl.ds(a, b - a)],
                                     arena.at[pl.ds(base + s0, rows), pl.ds(a, b - a)],
                                     sems.at[new_sem()])

    def pass_copy(h, j):
        u = pl.ds(lead + j * _RUN, _RUN)
        return pltpu.make_async_copy(ckv_hbm.at[pl.ds(h * NC, NC), u], arena.at[pl.ds(h * NC, NC), u],
                                     sems.at[h * (NJ - 1) + j])

    ckv_first = [rect(ckv_hbm, 0, h * NC, NC, 0, lead) for h in range(2)]
    ckv_last = [rect(ckv_hbm, 0, h * NC, NC, cuts[-2], _ROW) for h in range(2)]

    def wait_total(dst, sem):
        pltpu.make_async_copy(dst, dst, sems.at[sem]).wait()

    sem_wuv, sem_wo = new_sem(), new_sem()
    sem_ffn = [new_sem(2), new_sem(2)]
    PU = 4
    PPR = _ROW // PU
    BV = (NS * PPR - sum(pre_bursts)) // (2 * (NJ - 1))
    assert sum(pre_bursts) + BV * 2 * (NJ - 1) == NS * PPR

    def wuv_burst(k0, n, nspin, t):
        def body(u, t):
            k = k0 + u
            r, c = k // PPR, pl.ds((k % PPR) * PU, PU)
            pltpu.make_async_copy(wuv_hbm.at[r, c], arena.at[RV + r, c], sems.at[sem_wuv]).start()
            return lax.fori_loop(0, nspin, lambda i, t: t * 5 + i, t)
        return lax.fori_loop(0, n, body, t)

    npin = 1 + len(qk_split) + len(pv_split)
    FP = 8
    FPR = _ROW // FP
    n_ffn = npin // 2 * NJ
    full_rows = FR - 1
    ffn_part = n_ffn * FP - full_rows * _ROW
    assert npin % 2 == 0 and 0 < ffn_part < FU - full_rows * _ROW

    def ffn_pin(j, slot):
        src, base = ((w1_hbm, R1), (w2_hbm, R2))[slot % 2]
        k = j * (npin // 2) + slot // 2
        pltpu.make_async_copy(src.at[pl.ds(k * FP, FP)],
                              arena.at[base + k // FPR, pl.ds((k % FPR) * FP, FP)],
                              sems.at[sem_ffn[slot % 2] + k // (full_rows * FPR)]).start()

    def wo_pin(j, slot):
        u = pl.ds(slot * PU, PU)
        pltpu.make_async_copy(wo_hbm.at[j, u], arena.at[RO + j, u], sems.at[sem_wo]).start()

    wo_hi = npin * PU
    assert NJ == NS and UB <= wo_hi <= 2 * UB

    x_cp = pltpu.make_async_copy(x_hbm, x_v, sems.at[new_sem()])
    wq_cp = [rect(wq_hbm, RQ, 0, NS, a, b) for a, b in zip(cuts[:-1], cuts[1:])]
    wuk_cp = [rect(wuk_hbm, RK, 0, NS, a, b) for a, b in zip(cuts[:-1], cuts[1:])]
    ffn_cp = [pltpu.make_async_copy(src.at[pl.ds(n_ffn * FP, FU - n_ffn * FP)],
                                    arena.at[base + full_rows, pl.ds(ffn_part, FU - n_ffn * FP)],
                                    sems.at[new_sem()])
              for src, base in ((w1_hbm, R1), (w2_hbm, R2))]
    oc = [wo_hi] + [c for c in cuts if wo_hi < c]
    U3 = (NBLK - 1) * UB
    c3 = min(c for c in oc if c >= U3)
    HS = NS // 2
    wo_main = [rect(wo_hbm, RO, 0, NS, a, b) for a, b in zip(oc[:-1], oc[1:]) if b <= c3]
    wo_mxu = [rect(wo_hbm, RO, 0, HS, a, b) for a, b in zip(oc[:-1], oc[1:]) if a >= c3]
    tail = [(HS, 2, c3, U3, _ROW), (HS + 2, 1, c3, U3, _ROW), (NS - 1, 1, c3, U3, _ROW - 16),
            (NS - 1, 1, _ROW - 16, _ROW - 16, _ROW - 8), (NS - 1, 1, _ROW - 8, _ROW - 8, _ROW - 4),
            (NS - 1, 1, _ROW - 4, _ROW - 4, _ROW)]
    wo_tail = [rect(wo_hbm, RO, s0, n, a, b) for s0, n, a, _, b in tail]
    assert HS == 4 and c3 < _ROW - 16 and n_sem[0] <= sems.shape[0]

    queue = [x_cp] + wq_cp + wuk_cp + ffn_cp
    for h in range(2):
        queue += [ckv_first[h]] + [pass_copy(h, j) for j in range(NJ - 1)] + [ckv_last[h]]
    issued = [0]

    def issue(n):
        for cp in queue[issued[0]:issued[0] + n]:
            cp.start(priority=_LO)
        issued[0] = min(len(queue), issued[0] + n)

    issue(24)

    pre = [0, 0, jnp.int32(1)]

    def pre_burst():
        n = pre_bursts[pre[0]]
        if n:
            pre[2] = wuv_burst(pre[1], n, spin_pre, pre[2])
        pre[0] += 1
        pre[1] += n

    e_v[...] = jnp.where(_iota((128, EW), 1) // 8 == _iota((128, EW), 0), 1.0, 0.0).astype(_BF16)

    def diag(v):
        return jnp.where(_iota(v.shape, 1) % 8 == _iota(v.shape, 0) % 8, v, 0.0).astype(_BF16)

    def expand(v):
        R, K = v.shape
        st = jnp.concatenate([v[:, a * 128:(a + 1) * 128] for a in range(K // 128)], axis=0)
        ex = diag(_dot(st, e_v[...]))
        return jnp.concatenate([ex[a * R:(a + 1) * R] for a in range(K // 128)], axis=-1)

    pre_burst()
    x_cp.wait()
    x = x_v[...].astype(_F32)
    mu = jnp.mean(x, axis=-1, keepdims=True)
    xc = x - mu
    var = jnp.mean(xc * xc, axis=-1, keepdims=True)
    xn = (xc / jnp.sqrt(var + eps)).astype(_BF16)
    aq = expand(jnp.broadcast_to(xn, (16, M)))

    def block(base, b, rows=NS):
        return _halves(arena[base:base + rows, b * UB:(b + 1) * UB])

    def wait_block(cps, b, done):
        while done < len(cps) and cuts[done] < (b + 1) * UB:
            cps[done].wait()
            issue(1)
            done += 1
        return done

    BW = UB // 2 * 8
    SW = BW * NBLK
    qg = [jnp.zeros((16, _HW), _F32) for _ in range(2)]
    done = 0
    for b in range(NBLK):
        pre_burst()
        done = wait_block(wq_cp, b, done)
        lhs = jnp.concatenate([aq[:, s * SW + b * BW:s * SW + (b + 1) * BW] for s in range(NS)], axis=-1)
        for g, w in enumerate(block(RQ, b)):
            qg[g] = _dot(lhs, w) + qg[g]
    own = (_iota((16, _HW), 1) // D) == (_iota((16, _HW), 0) // 8)
    qg = [jnp.where(own, v, 0.0).astype(_BF16) for v in qg]

    scale = D ** -0.5
    tm = [[None] * NBLK for _ in range(2)]
    done = 0
    for b in range(NBLK):
        pre_burst()
        done = wait_block(wuk_cp, b, done)
        for g, w in enumerate(block(RK, b)):
            tm[g][b] = diag(_dot_t(qg[g], w) * scale)
    issue(len(queue))
    tn = [jnp.concatenate([tm[g][b][:, s * BW:(s + 1) * BW] for s in range(NS) for b in range(NBLK)], axis=-1)
          for g in range(2)]
    st = jnp.concatenate([tn[g][:, a * EW:(a + 1) * EW] for a in range(C // 128) for g in range(2)], axis=0)
    ql = _dot_t(st, e_v[...]).astype(_BF16)
    q_lat = jnp.concatenate([ql[a * H:(a + 1) * H] for a in range(C // 128)], axis=-1)
    pre_burst()

    R128 = 128 // (_RUN * 4)
    assert sum(qk_split) * R128 == NC and sum(pv_split) * R128 == NC

    def make_step(h, k0, pin_fn):
        def step(j, carry):
            m_old, l_old, acc, t = carry
            t = wuv_burst(k0 + j * BV, jnp.where(j == NJ - 1, 0, BV), spin_loop, t)
            pl.when(j < NJ - 1)(lambda: pass_copy(h, j).wait())
            pl.when(j == NJ - 1)(ckv_last[h].wait)
            slot = [0]

            def pin():
                pin_fn(j, slot[0])
                slot[0] += 1

            def keys(u0, n):
                r0 = h * NC + u0 * R128
                return _halves(arena[r0:r0 + n * R128, pl.ds(j * _RUN, _RUN)])

            pin()
            ss, u0 = [], 0
            for n in qk_split:
                ss.append(_dot_nt(q_lat, keys(u0, n)))
                pin()
                u0 += n
            s = jnp.concatenate(ss, axis=-1)
            m_new = jnp.maximum(m_old, jnp.max(s, axis=-1, keepdims=True))
            alpha = jnp.exp(m_old - m_new)
            p = jnp.exp(s - m_new)
            l_new = alpha * l_old + jnp.sum(p, axis=-1, keepdims=True)
            p = p.astype(_BF16)
            acc = alpha * acc
            u0 = 0
            for n in pv_split:
                acc = _dot_nn(p[:, u0 * 128:(u0 + n) * 128], keys(u0, n)) + acc
                pin()
                u0 += n
            return m_new, l_new, acc, t
        return step

    k0 = sum(pre_bursts)
    carry = (jnp.full((H, 1), -jnp.inf, _F32), jnp.zeros((H, 1), _F32), jnp.zeros((H, C), _F32), pre[2])
    ckv_first[0].wait()
    carry = lax.fori_loop(0, NJ, make_step(0, k0, ffn_pin), carry)

    for cp in wo_main + wo_mxu + wo_tail:
        cp.start(priority=_LO)
    for base, sem in zip((R1, R2), sem_ffn):
        wait_total(arena.at[pl.ds(base, full_rows)], sem)
        wait_total(arena.at[base + full_rows, pl.ds(0, ffn_part)], sem + 1)
    for cp in ffn_cp:
        cp.wait()

    def ffn_weight(base):
        v = arena[base:base + full_rows].reshape(full_rows * _ROW, 8, _HW)
        return _halves(jnp.concatenate([v, arena[base + full_rows, 0:FU - full_rows * _ROW]], axis=0))

    h1 = _silu(_dot_nt(jnp.broadcast_to(xn, (8, M)), ffn_weight(R1))).astype(_BF16)
    gate = _silu(_dot_nn(h1, ffn_weight(R2)))[0:1]

    ckv_first[1].wait()
    _, l_fin, acc, t = lax.fori_loop(0, NJ, make_step(1, k0 + BV * (NJ - 1), wo_pin), carry)
    sink[0] = t

    wait_total(arena.at[pl.ds(RV, NS)], sem_wuv)
    av = expand((acc / l_fin).astype(_BF16))
    cg = [_dot(av[g * 16:(g + 1) * 16], w) for g, w in enumerate(_halves(arena[RV:RV + NS]))]
    ctx = jnp.concatenate([cg[g][e * 8:(e + 1) * 8, e * D:(e + 1) * D]
                           for g in range(2) for e in range(2)], axis=0)
    ctx = ctx.astype(_BF16).astype(_F32)

    wait_total(arena.at[pl.ds(RO, NS), pl.ds(0, wo_hi)], sem_wo)
    row8 = _iota((8, D), 0)

    def wo_dot(b, rows):
        heads = [NBLK * s + b for s in range(rows)]
        lhs = jnp.concatenate([jnp.where(row8 == (h % 8), ctx[(h // 8) * 8:(h // 8) * 8 + 8, :], 0.0)
                               for h in heads], axis=-1).astype(_BF16)
        return _dot_nn(lhs, block(RO, b, rows))

    eye = _iota((D, D), 0) == _iota((D, D), 1)
    cols = [_dot(jnp.where(eye, jnp.broadcast_to(ctx[h:h + 1, :], (D, D)), 0.0).astype(_BF16),
                 jnp.ones((D, 128), _BF16)) for h in range(NBLK * HS + NBLK - 1, H, NBLK)]
    so8 = wo_dot(0, NS)
    for cp in wo_main:
        cp.wait()
    so8 = wo_dot(1, NS) + so8
    so8 = wo_dot(2, NS) + so8
    for cp in wo_mxu:
        cp.wait()
    so8 = wo_dot(3, HS) + so8
    for cp, (s0, n, _, a, b) in zip(wo_tail, tail):
        coef = jnp.concatenate([cols[s - HS][(a - U3) * 4:(b - U3) * 4] for s in range(s0, s0 + n)], axis=0)
        coef = jnp.concatenate([coef] * (M // 128), axis=-1)
        cp.wait()
        prod = coef * jnp.concatenate(_halves(arena[RO + s0:RO + s0 + n, a:b].astype(_F32)), axis=-1)
        for r in range(0, prod.shape[0], 8):
            so8 = so8 + prod[r:r + 8, :]
    s = jnp.sum(so8, axis=0, keepdims=True)

    o_ref[...] = (x + s * gate).astype(o_ref.dtype)


def _kernel(*refs, n_sems, **kw):
    pl.run_scoped(lambda sems: _body(*refs, sems, **kw),
                  pltpu.SemaphoreType.DMA((n_sems,)))


def _units(a):
    rows = a.shape[0]
    return a.reshape(rows // 8, 8, 2, _HW).transpose(0, 2, 1, 3).reshape(rows // 4, 8, _HW)


def _head_units(w):
    k, h, d = w.shape
    return w.reshape(k * h // 16, 2, 8, d).transpose(0, 2, 1, 3).reshape(-1, _ROW, 8, _HW)


def _forward(A_x, A_c_kv, A_w_q, A_w_uk, A_w_uv, A_w_o, B_w1, B_w2, *,
             lead=7, pre_bursts=(9, 14, 11, 11, 6, 14, 11, 11, 6, 9), spin_pre=12, spin_loop=17,
             qk_split=(3, 3, 3, 3, 2, 2), pv_split=(5, 5, 6)):
    B, SQ, M = A_x.shape
    _, SK, C = A_c_kv.shape
    _, H, D = A_w_q.shape
    F = B_w1.shape[1]
    assert B == 1 and SQ == 1 and H == 32 and 2 * D == _HW and M == 2 * _HW and C == 2 * _HW
    assert F % 8 == 0 and 0 < lead < _RUN
    dt = A_x.dtype
    rows = (SK + 4 * H * D) // 4 // _ROW + 2 * -(-(F // 4) // _ROW)
    kernel = functools.partial(
        _kernel, n_sems=64, H=H, D=D, M=M, C=C, lead=lead, pre_bursts=pre_bursts,
        spin_pre=spin_pre, spin_loop=spin_loop, qk_split=qk_split, pv_split=pv_split, eps=1e-5)
    any_spec = pl.BlockSpec(memory_space=pl.ANY)
    out = pl.pallas_call(
        kernel,
        in_specs=[any_spec] * 8,
        out_specs=pl.BlockSpec(memory_space=pltpu.VMEM),
        out_shape=jax.ShapeDtypeStruct((1, M), dt),
        scratch_shapes=[
            pltpu.VMEM((1, M), dt),
            pltpu.VMEM((rows, _ROW, 8, _HW), dt),
            pltpu.VMEM((128, 128 * 8), _BF16),
            pltpu.SMEM((1,), jnp.int32),
        ],
        compiler_params=pltpu.CompilerParams(vmem_limit_bytes=100 * 1024 * 1024),
    )(
        A_x.reshape(1, M),
        _units(A_c_kv.reshape(SK, C)).reshape(-1, _ROW, 8, _HW),
        _head_units(A_w_q),
        _head_units(A_w_uk),
        _head_units(A_w_uv),
        _units(A_w_o.reshape(H * D, M)).reshape(-1, _ROW, 8, _HW),
        _units(B_w1.T),
        _units(B_w2),
    )
    return out.reshape(B, SQ, M)


@jax.jit
def pallas_recurrent_scan__compressed_kv_cla__dense_activation_silu__decode_kernel(
    A_x: jax.Array,
    A_c_kv: jax.Array,
    A_w_q: jax.Array,
    A_w_uk: jax.Array,
    A_w_uv: jax.Array,
    A_w_o: jax.Array,
    B_x: jax.Array,
    B_w1: jax.Array,
    B_w2: jax.Array,
):
    return _forward(A_x, A_c_kv, A_w_q, A_w_uk, A_w_uv, A_w_o, B_w1, B_w2)
```

```python
import functools

import jax
import jax.numpy as jnp
from jax import lax
import jax.experimental.pallas as pl
import jax.experimental.pallas.tpu as pltpu

_F32 = jnp.float32
_BF16 = jnp.bfloat16
_LO = 1
_HW = 256
_RUN = 16
_ROW = 128


def _silu(v):
    return v / (1.0 + jnp.exp(-v))


def _rnd(v):
    return v.astype(_BF16).astype(_F32)


def _iota(shape, dim):
    return lax.broadcasted_iota(jnp.int32, shape, dim)


def _halves(v):
    v = v.reshape(-1, 2, 8, _HW)
    return [v[:, e].reshape(-1, _HW) for e in range(2)]


def _dot(a, b):
    return jnp.dot(a, b, preferred_element_type=_F32)


def _dot_t(a, b):
    return lax.dot_general(a, b, (((1,), (1,)), ((), ())), preferred_element_type=_F32)


def _dot_nt(a, kh):
    return _dot_t(a[:, :_HW], kh[0]) + _dot_t(a[:, _HW:], kh[1])


def _dot_nn(a, kh):
    return jnp.concatenate([_dot(a, k) for k in kh], axis=-1)


def _body(x_hbm, ckv_hbm, wq_hbm, wuk_hbm, wuv_hbm, wo_hbm, w1_hbm, w2_hbm,
          o_ref, x_v, arena, e_v, sink, sems,
          *, H, D, M, C, lead, pre_bursts, spin_pre, spin_loop, qk_split, pv_split, eps):
    NC = ckv_hbm.shape[0] // 2
    NS = wq_hbm.shape[0]
    FU = w1_hbm.shape[0]
    FR = -(-FU // _ROW)
    RQ = 2 * NC
    RK, RV, RO = RQ + NS, RQ + 2 * NS, RQ + 3 * NS
    R1 = RO + NS
    R2 = R1 + FR
    NJ = _ROW // _RUN
    NBLK = 4
    UB = _ROW // NBLK
    EW = 128 * 8
    cuts = [0] + list(range(lead, _ROW, _RUN)) + [_ROW]

    n_sem = [2 * (NJ - 1)]

    def new_sem(n=1):
        n_sem[0] += n
        return n_sem[0] - n

    def rect(src, base, s0, rows, a, b):
        return pltpu.make_async_copy(src.at[pl.ds(s0, rows), pl.ds(a, b - a)],
                                     arena.at[pl.ds(base + s0, rows), pl.ds(a, b - a)],
                                     sems.at[new_sem()])

    def pass_copy(h, j):
        u = pl.ds(lead + j * _RUN, _RUN)
        return pltpu.make_async_copy(ckv_hbm.at[pl.ds(h * NC, NC), u], arena.at[pl.ds(h * NC, NC), u],
                                     sems.at[h * (NJ - 1) + j])

    ckv_first = [rect(ckv_hbm, 0, h * NC, NC, 0, lead) for h in range(2)]
    ckv_last = [rect(ckv_hbm, 0, h * NC, NC, cuts[-2], _ROW) for h in range(2)]

    def wait_total(dst, sem):
        pltpu.make_async_copy(dst, dst, sems.at[sem]).wait()

    sem_wuv, sem_wo = new_sem(), new_sem()
    sem_ffn = [new_sem(2), new_sem(2)]
    PU = 4
    PPR = _ROW // PU
    BV = (NS * PPR - sum(pre_bursts)) // (2 * (NJ - 1))
    assert sum(pre_bursts) + BV * 2 * (NJ - 1) == NS * PPR

    def wuv_burst(k0, n, nspin, t):
        def body(u, t):
            k = k0 + u
            r, c = k // PPR, pl.ds((k % PPR) * PU, PU)
            pltpu.make_async_copy(wuv_hbm.at[r, c], arena.at[RV + r, c], sems.at[sem_wuv]).start()
            return lax.fori_loop(0, nspin, lambda i, t: t * 5 + i, t)
        return lax.fori_loop(0, n, body, t)

    npin = 1 + len(qk_split) + len(pv_split)
    FP = 8
    FPR = _ROW // FP
    n_ffn = npin // 2 * NJ
    full_rows = FR - 1
    ffn_part = n_ffn * FP - full_rows * _ROW
    assert npin % 2 == 0 and 0 < ffn_part < FU - full_rows * _ROW

    def ffn_pin(j, slot):
        src, base = ((w1_hbm, R1), (w2_hbm, R2))[slot % 2]
        k = j * (npin // 2) + slot // 2
        pltpu.make_async_copy(src.at[pl.ds(k * FP, FP)],
                              arena.at[base + k // FPR, pl.ds((k % FPR) * FP, FP)],
                              sems.at[sem_ffn[slot % 2] + k // (full_rows * FPR)]).start()

    def wo_pin(j, slot):
        u = pl.ds(slot * PU, PU)
        pltpu.make_async_copy(wo_hbm.at[j, u], arena.at[RO + j, u], sems.at[sem_wo]).start()

    wo_hi = npin * PU
    assert NJ == NS and UB <= wo_hi <= 2 * UB

    x_cp = pltpu.make_async_copy(x_hbm, x_v, sems.at[new_sem()])
    wq_cp = [rect(wq_hbm, RQ, 0, NS, a, b) for a, b in zip(cuts[:-1], cuts[1:])]
    wuk_cp = [rect(wuk_hbm, RK, 0, NS, a, b) for a, b in zip(cuts[:-1], cuts[1:])]
    ffn_cp = [pltpu.make_async_copy(src.at[pl.ds(n_ffn * FP, FU - n_ffn * FP)],
                                    arena.at[base + full_rows, pl.ds(ffn_part, FU - n_ffn * FP)],
                                    sems.at[new_sem()])
              for src, base in ((w1_hbm, R1), (w2_hbm, R2))]
    oc = [wo_hi] + [c for c in cuts if wo_hi < c]
    U3 = (NBLK - 1) * UB
    c3 = min(c for c in oc if c >= U3)
    HS = NS // 2
    wo_main = [rect(wo_hbm, RO, 0, NS, a, b) for a, b in zip(oc[:-1], oc[1:]) if b <= c3]
    wo_mxu = [rect(wo_hbm, RO, 0, HS, a, b) for a, b in zip(oc[:-1], oc[1:]) if a >= c3]
    tail = [(HS, 2, c3, U3, _ROW), (HS + 2, 1, c3, U3, _ROW), (NS - 1, 1, c3, U3, _ROW - 16),
            (NS - 1, 1, _ROW - 16, _ROW - 16, _ROW - 8), (NS - 1, 1, _ROW - 8, _ROW - 8, _ROW - 4),
            (NS - 1, 1, _ROW - 4, _ROW - 4, _ROW)]
    wo_tail = [rect(wo_hbm, RO, s0, n, a, b) for s0, n, a, _, b in tail]
    assert HS == 4 and c3 < _ROW - 16 and n_sem[0] <= sems.shape[0]

    queue = [x_cp] + wq_cp + wuk_cp + ffn_cp
    for h in range(2):
        queue += [ckv_first[h]] + [pass_copy(h, j) for j in range(NJ - 1)] + [ckv_last[h]]
    issued = [0]

    def issue(n):
        for cp in queue[issued[0]:issued[0] + n]:
            cp.start(priority=_LO)
        issued[0] = min(len(queue), issued[0] + n)

    issue(24)

    pre = [0, 0, jnp.int32(1)]

    def pre_burst():
        n = pre_bursts[pre[0]]
        if n:
            pre[2] = wuv_burst(pre[1], n, spin_pre, pre[2])
        pre[0] += 1
        pre[1] += n

    e_v[...] = jnp.where(_iota((128, EW), 1) // 8 == _iota((128, EW), 0), 1.0, 0.0).astype(_BF16)

    def diag(v):
        return jnp.where(_iota(v.shape, 1) % 8 == _iota(v.shape, 0) % 8, v, 0.0).astype(_BF16)

    def expand(v):
        R, K = v.shape
        st = jnp.concatenate([v[:, a * 128:(a + 1) * 128] for a in range(K // 128)], axis=0)
        ex = diag(_dot(st, e_v[...]))
        return jnp.concatenate([ex[a * R:(a + 1) * R] for a in range(K // 128)], axis=-1)

    pre_burst()
    x_cp.wait()
    x = x_v[...].astype(_F32)
    mu = jnp.mean(x, axis=-1, keepdims=True)
    var = jnp.mean((x - mu) * (x - mu), axis=-1, keepdims=True)
    xn = (_rnd(x - _rnd(mu)) / _rnd(jnp.sqrt(_rnd(_rnd(var) + eps)))).astype(_BF16)
    aq = expand(jnp.broadcast_to(xn, (16, M)))

    def block(base, b, rows=NS):
        return _halves(arena[base:base + rows, b * UB:(b + 1) * UB])

    def wait_block(cps, b, done):
        while done < len(cps) and cuts[done] < (b + 1) * UB:
            cps[done].wait()
            issue(1)
            done += 1
        return done

    BW = UB // 2 * 8
    SW = BW * NBLK
    qg = [jnp.zeros((16, _HW), _F32) for _ in range(2)]
    done = 0
    for b in range(NBLK):
        pre_burst()
        done = wait_block(wq_cp, b, done)
        lhs = jnp.concatenate([aq[:, s * SW + b * BW:s * SW + (b + 1) * BW] for s in range(NS)], axis=-1)
        for g, w in enumerate(block(RQ, b)):
            qg[g] = _dot(lhs, w) + qg[g]
    own = (_iota((16, _HW), 1) // D) == (_iota((16, _HW), 0) // 8)
    qg = [jnp.where(own, v, 0.0).astype(_BF16) for v in qg]

    scale = D ** -0.5
    tm = [[None] * NBLK for _ in range(2)]
    done = 0
    for b in range(NBLK):
        pre_burst()
        done = wait_block(wuk_cp, b, done)
        for g, w in enumerate(block(RK, b)):
            tm[g][b] = diag(_dot_t(qg[g], w) * scale)
    issue(len(queue))
    tn = [jnp.concatenate([tm[g][b][:, s * BW:(s + 1) * BW] for s in range(NS) for b in range(NBLK)], axis=-1)
          for g in range(2)]
    st = jnp.concatenate([tn[g][:, a * EW:(a + 1) * EW] for a in range(C // 128) for g in range(2)], axis=0)
    ql = _dot_t(st, e_v[...]).astype(_BF16)
    q_lat = jnp.concatenate([ql[a * H:(a + 1) * H] for a in range(C // 128)], axis=-1)
    pre_burst()

    R128 = 128 // (_RUN * 4)
    assert sum(qk_split) * R128 == NC and sum(pv_split) * R128 == NC

    def make_step(h, k0, pin_fn):
        def step(j, carry):
            m_old, l_old, acc, t = carry
            t = wuv_burst(k0 + j * BV, jnp.where(j == NJ - 1, 0, BV), spin_loop, t)
            pl.when(j < NJ - 1)(lambda: pass_copy(h, j).wait())
            pl.when(j == NJ - 1)(ckv_last[h].wait)
            slot = [0]

            def pin():
                pin_fn(j, slot[0])
                slot[0] += 1

            def keys(u0, n):
                r0 = h * NC + u0 * R128
                return _halves(arena[r0:r0 + n * R128, pl.ds(j * _RUN, _RUN)])

            pin()
            ss, u0 = [], 0
            for n in qk_split:
                ss.append(_dot_nt(q_lat, keys(u0, n)))
                pin()
                u0 += n
            s = jnp.concatenate(ss, axis=-1)
            m_new = jnp.maximum(m_old, jnp.max(s, axis=-1, keepdims=True))
            alpha = jnp.exp(m_old - m_new)
            p = jnp.exp(s - m_new)
            l_new = alpha * l_old + jnp.sum(p, axis=-1, keepdims=True)
            p = p.astype(_BF16)
            acc = alpha * acc
            u0 = 0
            for n in pv_split:
                acc = _dot_nn(p[:, u0 * 128:(u0 + n) * 128], keys(u0, n)) + acc
                pin()
                u0 += n
            return m_new, l_new, acc, t
        return step

    k0 = sum(pre_bursts)
    carry = (jnp.full((H, 1), -jnp.inf, _F32), jnp.zeros((H, 1), _F32), jnp.zeros((H, C), _F32), pre[2])
    ckv_first[0].wait()
    carry = lax.fori_loop(0, NJ, make_step(0, k0, ffn_pin), carry)

    for cp in wo_main + wo_mxu + wo_tail:
        cp.start(priority=_LO)
    for base, sem in zip((R1, R2), sem_ffn):
        wait_total(arena.at[pl.ds(base, full_rows)], sem)
        wait_total(arena.at[base + full_rows, pl.ds(0, ffn_part)], sem + 1)
    for cp in ffn_cp:
        cp.wait()

    def ffn_weight(base):
        v = arena[base:base + full_rows].reshape(full_rows * _ROW, 8, _HW)
        return _halves(jnp.concatenate([v, arena[base + full_rows, 0:FU - full_rows * _ROW]], axis=0))

    h1 = _silu(_rnd(_dot_nt(jnp.broadcast_to(xn, (8, M)), ffn_weight(R1)))).astype(_BF16)
    gate = _silu(_rnd(_dot_nn(h1, ffn_weight(R2))))
    x8 = jnp.broadcast_to(x, (8, M))

    ckv_first[1].wait()
    _, l_fin, acc, t = lax.fori_loop(0, NJ, make_step(1, k0 + BV * (NJ - 1), wo_pin), carry)
    sink[0] = t

    wait_total(arena.at[pl.ds(RV, NS)], sem_wuv)
    av = expand((acc / l_fin).astype(_BF16))
    cg = [_dot(av[g * 16:(g + 1) * 16], w) for g, w in enumerate(_halves(arena[RV:RV + NS]))]
    ctx = jnp.concatenate([cg[g][e * 8:(e + 1) * 8, e * D:(e + 1) * D]
                           for g in range(2) for e in range(2)], axis=0)
    ctx = _rnd(ctx)

    wait_total(arena.at[pl.ds(RO, NS), pl.ds(0, wo_hi)], sem_wo)
    row8 = _iota((8, D), 0)

    def wo_dot(b, rows):
        heads = [NBLK * s + b for s in range(rows)]
        lhs = jnp.concatenate([jnp.where(row8 == (h % 8), ctx[(h // 8) * 8:(h // 8) * 8 + 8, :], 0.0)
                               for h in heads], axis=-1).astype(_BF16)
        return _dot_nn(lhs, block(RO, b, rows))

    eye = _iota((D, D), 0) == _iota((D, D), 1)
    cols = [_dot(jnp.where(eye, jnp.broadcast_to(ctx[h:h + 1, :], (D, D)), 0.0).astype(_BF16),
                 jnp.ones((D, 128), _BF16)) for h in range(NBLK * HS + NBLK - 1, H, NBLK)]
    so8 = wo_dot(0, NS)
    for cp in wo_main:
        cp.wait()
    so8 = wo_dot(1, NS) + so8
    so8 = wo_dot(2, NS) + so8
    for cp in wo_mxu:
        cp.wait()
    so8 = wo_dot(3, HS) + so8
    for cp, (s0, n, _, a, b) in zip(wo_tail, tail):
        coef = jnp.concatenate([cols[s - HS][(a - U3) * 4:(b - U3) * 4] for s in range(s0, s0 + n)], axis=0)
        coef = jnp.concatenate([coef] * (M // 128), axis=-1)
        cp.wait()
        prod = coef * jnp.concatenate(_halves(arena[RO + s0:RO + s0 + n, a:b].astype(_F32)), axis=-1)
        for r in range(0, prod.shape[0], 8):
            so8 = so8 + prod[r:r + 8, :]
    s = jnp.sum(so8, axis=0, keepdims=True)

    o_ref[...] = (x8 + s * gate)[0:1].astype(o_ref.dtype)


def _kernel(*refs, n_sems, **kw):
    pl.run_scoped(lambda sems: _body(*refs, sems, **kw),
                  pltpu.SemaphoreType.DMA((n_sems,)))


def _units(a):
    rows = a.shape[0]
    return a.reshape(rows // 8, 8, 2, _HW).transpose(0, 2, 1, 3).reshape(rows // 4, 8, _HW)


def _head_units(w):
    k, h, d = w.shape
    return w.reshape(k * h // 16, 2, 8, d).transpose(0, 2, 1, 3).reshape(-1, _ROW, 8, _HW)


def _forward(A_x, A_c_kv, A_w_q, A_w_uk, A_w_uv, A_w_o, B_w1, B_w2, *,
             lead=7, pre_bursts=(9, 14, 11, 11, 6, 14, 11, 11, 6, 9), spin_pre=12, spin_loop=17,
             qk_split=(3, 3, 3, 3, 2, 2), pv_split=(5, 5, 6)):
    B, SQ, M = A_x.shape
    _, SK, C = A_c_kv.shape
    _, H, D = A_w_q.shape
    F = B_w1.shape[1]
    assert B == 1 and SQ == 1 and H == 32 and 2 * D == _HW and M == 2 * _HW and C == 2 * _HW
    assert F % 8 == 0 and 0 < lead < _RUN
    dt = A_x.dtype
    rows = (SK + 4 * H * D) // 4 // _ROW + 2 * -(-(F // 4) // _ROW)
    kernel = functools.partial(
        _kernel, n_sems=64, H=H, D=D, M=M, C=C, lead=lead, pre_bursts=pre_bursts,
        spin_pre=spin_pre, spin_loop=spin_loop, qk_split=qk_split, pv_split=pv_split, eps=1e-5)
    any_spec = pl.BlockSpec(memory_space=pl.ANY)
    out = pl.pallas_call(
        kernel,
        in_specs=[any_spec] * 8,
        out_specs=pl.BlockSpec(memory_space=pltpu.VMEM),
        out_shape=jax.ShapeDtypeStruct((1, M), dt),
        scratch_shapes=[
            pltpu.VMEM((1, M), dt),
            pltpu.VMEM((rows, _ROW, 8, _HW), dt),
            pltpu.VMEM((128, 128 * 8), _BF16),
            pltpu.SMEM((1,), jnp.int32),
        ],
        compiler_params=pltpu.CompilerParams(vmem_limit_bytes=100 * 1024 * 1024),
    )(
        A_x.reshape(1, M),
        _units(A_c_kv.reshape(SK, C)).reshape(-1, _ROW, 8, _HW),
        _head_units(A_w_q),
        _head_units(A_w_uk),
        _head_units(A_w_uv),
        _units(A_w_o.reshape(H * D, M)).reshape(-1, _ROW, 8, _HW),
        _units(B_w1.T),
        _units(B_w2),
    )
    return out.reshape(B, SQ, M)


@jax.jit
def pallas_recurrent_scan__compressed_kv_cla__dense_activation_silu__decode_kernel(
    A_x: jax.Array,
    A_c_kv: jax.Array,
    A_w_q: jax.Array,
    A_w_uk: jax.Array,
    A_w_uv: jax.Array,
    A_w_o: jax.Array,
    B_x: jax.Array,
    B_w1: jax.Array,
    B_w2: jax.Array,
):
    return _forward(A_x, A_c_kv, A_w_q, A_w_uk, A_w_uv, A_w_o, B_w1, B_w2)
```

```python
import functools

import jax
import jax.numpy as jnp
from jax import lax
import jax.experimental.pallas as pl
import jax.experimental.pallas.tpu as pltpu

_F32 = jnp.float32
_BF16 = jnp.bfloat16
_LO = 1
_HW = 256
_RUN = 16
_ROW = 128


def _silu(v):
    return v / (1.0 + jnp.exp(-v))


def _rnd(v):
    return v.astype(_BF16).astype(_F32)


def _iota(shape, dim):
    return lax.broadcasted_iota(jnp.int32, shape, dim)


def _halves(v):
    v = v.reshape(-1, 2, 8, _HW)
    return [v[:, e].reshape(-1, _HW) for e in range(2)]


def _dot(a, b):
    return jnp.dot(a, b, preferred_element_type=_F32)


def _dot_t(a, b):
    return lax.dot_general(a, b, (((1,), (1,)), ((), ())), preferred_element_type=_F32)


def _dot_nt(a, kh):
    return _dot_t(a[:, :_HW], kh[0]) + _dot_t(a[:, _HW:], kh[1])


def _dot_nn(a, kh):
    return jnp.concatenate([_dot(a, k) for k in kh], axis=-1)


def _body(x_hbm, ckv_hbm, wq_hbm, wuk_hbm, wuv_hbm, wo_hbm, w1_hbm, w2_hbm,
          o_ref, x_v, arena, e_v, sink, sems,
          *, H, D, M, C, lead, pre_bursts, spin_pre, spin_loop, qk_split, pv_split, eps):
    NC = ckv_hbm.shape[0] // 2
    NS = wq_hbm.shape[0]
    FU = w1_hbm.shape[0]
    FR = -(-FU // _ROW)
    RQ = 2 * NC
    RK, RV, RO = RQ + NS, RQ + 2 * NS, RQ + 3 * NS
    R1 = RO + NS
    R2 = R1 + FR
    NJ = _ROW // _RUN
    NBLK = 4
    UB = _ROW // NBLK
    EW = 128 * 8
    cuts = [0] + list(range(lead, _ROW, _RUN)) + [_ROW]

    n_sem = [2 * (NJ - 1)]

    def new_sem(n=1):
        n_sem[0] += n
        return n_sem[0] - n

    def rect(src, base, s0, rows, a, b):
        return pltpu.make_async_copy(src.at[pl.ds(s0, rows), pl.ds(a, b - a)],
                                     arena.at[pl.ds(base + s0, rows), pl.ds(a, b - a)],
                                     sems.at[new_sem()])

    def pass_copy(h, j):
        u = pl.ds(lead + j * _RUN, _RUN)
        return pltpu.make_async_copy(ckv_hbm.at[pl.ds(h * NC, NC), u], arena.at[pl.ds(h * NC, NC), u],
                                     sems.at[h * (NJ - 1) + j])

    ckv_first = [rect(ckv_hbm, 0, h * NC, NC, 0, lead) for h in range(2)]
    ckv_last = [rect(ckv_hbm, 0, h * NC, NC, cuts[-2], _ROW) for h in range(2)]

    def wait_total(dst, sem):
        pltpu.make_async_copy(dst, dst, sems.at[sem]).wait()

    sem_wuv, sem_wo = new_sem(), new_sem()
    sem_ffn = [new_sem(2), new_sem(2)]
    BV = (NS * _ROW - sum(pre_bursts)) // (2 * (NJ - 1))
    assert sum(pre_bursts) + BV * 2 * (NJ - 1) == NS * _ROW

    def wuv_burst(k0, n, nspin, t):
        def body(u, t):
            k = k0 + u
            r, c = k // _ROW, pl.ds(k % _ROW, 1)
            pltpu.make_async_copy(wuv_hbm.at[r, c], arena.at[RV + r, c], sems.at[sem_wuv]).start()
            return lax.fori_loop(0, nspin, lambda i, t: t * 5 + i, t)
        return lax.fori_loop(0, n, body, t)

    npin = 1 + len(qk_split) + len(pv_split)
    FP, PU = 8, 4
    FPR = _ROW // FP
    n_ffn = npin // 2 * NJ
    full_rows = FR - 1
    ffn_part = n_ffn * FP - full_rows * _ROW
    assert npin % 2 == 0 and 0 < ffn_part < FU - full_rows * _ROW

    def ffn_pin(j, slot):
        src, base = ((w1_hbm, R1), (w2_hbm, R2))[slot % 2]
        k = j * (npin // 2) + slot // 2
        pltpu.make_async_copy(src.at[pl.ds(k * FP, FP)],
                              arena.at[base + k // FPR, pl.ds((k % FPR) * FP, FP)],
                              sems.at[sem_ffn[slot % 2] + k // (full_rows * FPR)]).start()

    def wo_pin(j, slot):
        u = pl.ds(slot * PU, PU)
        pltpu.make_async_copy(wo_hbm.at[j, u], arena.at[RO + j, u], sems.at[sem_wo]).start()

    wo_hi = npin * PU
    assert NJ == NS and UB <= wo_hi <= 2 * UB

    x_cp = pltpu.make_async_copy(x_hbm, x_v, sems.at[new_sem()])
    wq_cp = [rect(wq_hbm, RQ, 0, NS, a, b) for a, b in zip(cuts[:-1], cuts[1:])]
    wuk_cp = [rect(wuk_hbm, RK, 0, NS, a, b) for a, b in zip(cuts[:-1], cuts[1:])]
    ffn_cp = [pltpu.make_async_copy(src.at[pl.ds(n_ffn * FP, FU - n_ffn * FP)],
                                    arena.at[base + full_rows, pl.ds(ffn_part, FU - n_ffn * FP)],
                                    sems.at[new_sem()])
              for src, base in ((w1_hbm, R1), (w2_hbm, R2))]
    oc = [wo_hi] + [c for c in cuts if wo_hi < c]
    U3 = (NBLK - 1) * UB
    c3 = min(c for c in oc if c >= U3)
    HS = NS // 2
    wo_main = [rect(wo_hbm, RO, 0, NS, a, b) for a, b in zip(oc[:-1], oc[1:]) if b <= c3]
    wo_mxu = [rect(wo_hbm, RO, 0, HS, a, b) for a, b in zip(oc[:-1], oc[1:]) if a >= c3]
    tail = [(HS, 2, c3, U3, _ROW), (HS + 2, 1, c3, U3, _ROW), (NS - 1, 1, c3, U3, _ROW - 16),
            (NS - 1, 1, _ROW - 16, _ROW - 16, _ROW - 8), (NS - 1, 1, _ROW - 8, _ROW - 8, _ROW - 4),
            (NS - 1, 1, _ROW - 4, _ROW - 4, _ROW)]
    wo_tail = [rect(wo_hbm, RO, s0, n, a, b) for s0, n, a, _, b in tail]
    assert HS == 4 and c3 < _ROW - 16 and n_sem[0] <= sems.shape[0]

    queue = [x_cp] + wq_cp + wuk_cp + ffn_cp
    for h in range(2):
        queue += [ckv_first[h]] + [pass_copy(h, j) for j in range(NJ - 1)] + [ckv_last[h]]
    issued = [0]

    def issue(n):
        for cp in queue[issued[0]:issued[0] + n]:
            cp.start(priority=_LO)
        issued[0] = min(len(queue), issued[0] + n)

    issue(24)

    pre = [0, 0, jnp.int32(1)]

    def pre_burst():
        n = pre_bursts[pre[0]]
        if n:
            pre[2] = wuv_burst(pre[1], n, spin_pre, pre[2])
        pre[0] += 1
        pre[1] += n

    e_v[...] = jnp.where(_iota((128, EW), 1) // 8 == _iota((128, EW), 0), 1.0, 0.0).astype(_BF16)

    def diag(v):
        return jnp.where(_iota(v.shape, 1) % 8 == _iota(v.shape, 0) % 8, v, 0.0).astype(_BF16)

    def expand(v):
        R, K = v.shape
        st = jnp.concatenate([v[:, a * 128:(a + 1) * 128] for a in range(K // 128)], axis=0)
        ex = diag(_dot(st, e_v[...]))
        return jnp.concatenate([ex[a * R:(a + 1) * R] for a in range(K // 128)], axis=-1)

    pre_burst()
    x_cp.wait()
    x = x_v[...].astype(_F32)
    mu = jnp.mean(x, axis=-1, keepdims=True)
    var = jnp.mean((x - mu) * (x - mu), axis=-1, keepdims=True)
    xn = (_rnd(x - _rnd(mu)) / _rnd(jnp.sqrt(_rnd(_rnd(var) + eps)))).astype(_BF16)
    aq = expand(jnp.broadcast_to(xn, (16, M)))

    def block(base, b, rows=NS):
        return _halves(arena[base:base + rows, b * UB:(b + 1) * UB])

    def wait_block(cps, b, done):
        while done < len(cps) and cuts[done] < (b + 1) * UB:
            cps[done].wait()
            issue(1)
            done += 1
        return done

    BW = UB // 2 * 8
    SW = BW * NBLK
    qg = [jnp.zeros((16, _HW), _F32) for _ in range(2)]
    done = 0
    for b in range(NBLK):
        pre_burst()
        done = wait_block(wq_cp, b, done)
        lhs = jnp.concatenate([aq[:, s * SW + b * BW:s * SW + (b + 1) * BW] for s in range(NS)], axis=-1)
        for g, w in enumerate(block(RQ, b)):
            qg[g] = _dot(lhs, w) + qg[g]
    own = (_iota((16, _HW), 1) // D) == (_iota((16, _HW), 0) // 8)
    qg = [jnp.where(own, v, 0.0).astype(_BF16) for v in qg]

    scale = D ** -0.5
    tm = [[None] * NBLK for _ in range(2)]
    done = 0
    for b in range(NBLK):
        pre_burst()
        done = wait_block(wuk_cp, b, done)
        for g, w in enumerate(block(RK, b)):
            tm[g][b] = diag(_dot_t(qg[g], w) * scale)
    issue(len(queue))
    tn = [jnp.concatenate([tm[g][b][:, s * BW:(s + 1) * BW] for s in range(NS) for b in range(NBLK)], axis=-1)
          for g in range(2)]
    st = jnp.concatenate([tn[g][:, a * EW:(a + 1) * EW] for a in range(C // 128) for g in range(2)], axis=0)
    ql = _dot_t(st, e_v[...]).astype(_BF16)
    q_lat = jnp.concatenate([ql[a * H:(a + 1) * H] for a in range(C // 128)], axis=-1)
    pre_burst()

    R128 = 128 // (_RUN * 4)
    assert sum(qk_split) * R128 == NC and sum(pv_split) * R128 == NC

    def make_step(h, k0, pin_fn):
        def step(j, carry):
            m_old, l_old, acc, t = carry
            t = wuv_burst(k0 + j * BV, jnp.where(j == NJ - 1, 0, BV), spin_loop, t)
            pl.when(j < NJ - 1)(lambda: pass_copy(h, j).wait())
            pl.when(j == NJ - 1)(ckv_last[h].wait)
            slot = [0]

            def pin():
                pin_fn(j, slot[0])
                slot[0] += 1

            def keys(u0, n):
                r0 = h * NC + u0 * R128
                return _halves(arena[r0:r0 + n * R128, pl.ds(j * _RUN, _RUN)])

            pin()
            ss, u0 = [], 0
            for n in qk_split:
                ss.append(_dot_nt(q_lat, keys(u0, n)))
                pin()
                u0 += n
            s = jnp.concatenate(ss, axis=-1)
            m_new = jnp.maximum(m_old, jnp.max(s, axis=-1, keepdims=True))
            alpha = jnp.exp(m_old - m_new)
            p = jnp.exp(s - m_new)
            l_new = alpha * l_old + jnp.sum(p, axis=-1, keepdims=True)
            p = p.astype(_BF16)
            acc = alpha * acc
            u0 = 0
            for n in pv_split:
                acc = _dot_nn(p[:, u0 * 128:(u0 + n) * 128], keys(u0, n)) + acc
                pin()
                u0 += n
            return m_new, l_new, acc, t
        return step

    k0 = sum(pre_bursts)
    carry = (jnp.full((H, 1), -jnp.inf, _F32), jnp.zeros((H, 1), _F32), jnp.zeros((H, C), _F32), pre[2])
    ckv_first[0].wait()
    carry = lax.fori_loop(0, NJ, make_step(0, k0, ffn_pin), carry)

    for cp in wo_main + wo_mxu + wo_tail:
        cp.start(priority=_LO)
    for base, sem in zip((R1, R2), sem_ffn):
        wait_total(arena.at[pl.ds(base, full_rows)], sem)
        wait_total(arena.at[base + full_rows, pl.ds(0, ffn_part)], sem + 1)
    for cp in ffn_cp:
        cp.wait()

    def ffn_weight(base):
        v = arena[base:base + full_rows].reshape(full_rows * _ROW, 8, _HW)
        return _halves(jnp.concatenate([v, arena[base + full_rows, 0:FU - full_rows * _ROW]], axis=0))

    h1 = _silu(_rnd(_dot_nt(jnp.broadcast_to(xn, (8, M)), ffn_weight(R1)))).astype(_BF16)
    gate = _silu(_rnd(_dot_nn(h1, ffn_weight(R2))))
    x8 = jnp.broadcast_to(x, (8, M))

    ckv_first[1].wait()
    _, l_fin, acc, t = lax.fori_loop(0, NJ, make_step(1, k0 + BV * (NJ - 1), wo_pin), carry)
    sink[0] = t

    wait_total(arena.at[pl.ds(RV, NS)], sem_wuv)
    av = expand((acc / l_fin).astype(_BF16))
    cg = [_dot(av[g * 16:(g + 1) * 16], w) for g, w in enumerate(_halves(arena[RV:RV + NS]))]
    ctx = jnp.concatenate([cg[g][e * 8:(e + 1) * 8, e * D:(e + 1) * D]
                           for g in range(2) for e in range(2)], axis=0)
    ctx = _rnd(ctx)

    wait_total(arena.at[pl.ds(RO, NS), pl.ds(0, wo_hi)], sem_wo)
    row8 = _iota((8, D), 0)

    def wo_dot(b, rows):
        heads = [NBLK * s + b for s in range(rows)]
        lhs = jnp.concatenate([jnp.where(row8 == (h % 8), ctx[(h // 8) * 8:(h // 8) * 8 + 8, :], 0.0)
                               for h in heads], axis=-1).astype(_BF16)
        return _dot_nn(lhs, block(RO, b, rows))

    eye = _iota((D, D), 0) == _iota((D, D), 1)
    cols = [_dot(jnp.where(eye, jnp.broadcast_to(ctx[h:h + 1, :], (D, D)), 0.0).astype(_BF16),
                 jnp.ones((D, 128), _BF16)) for h in range(NBLK * HS + NBLK - 1, H, NBLK)]
    so8 = wo_dot(0, NS)
    for cp in wo_main:
        cp.wait()
    so8 = wo_dot(1, NS) + so8
    so8 = wo_dot(2, NS) + so8
    for cp in wo_mxu:
        cp.wait()
    so8 = wo_dot(3, HS) + so8
    for cp, (s0, n, _, a, b) in zip(wo_tail, tail):
        coef = jnp.concatenate([cols[s - HS][(a - U3) * 4:(b - U3) * 4] for s in range(s0, s0 + n)], axis=0)
        coef = jnp.concatenate([coef] * (M // 128), axis=-1)
        cp.wait()
        prod = coef * jnp.concatenate(_halves(arena[RO + s0:RO + s0 + n, a:b].astype(_F32)), axis=-1)
        for r in range(0, prod.shape[0], 8):
            so8 = so8 + prod[r:r + 8, :]
    s = jnp.sum(so8, axis=0, keepdims=True)

    o_ref[...] = (x8 + s * gate)[0:1].astype(o_ref.dtype)


def _kernel(*refs, n_sems, **kw):
    pl.run_scoped(lambda sems: _body(*refs, sems, **kw),
                  pltpu.SemaphoreType.DMA((n_sems,)))


def _units(a):
    rows = a.shape[0]
    return a.reshape(rows // 8, 8, 2, _HW).transpose(0, 2, 1, 3).reshape(rows // 4, 8, _HW)


def _head_units(w):
    k, h, d = w.shape
    return w.reshape(k * h // 16, 2, 8, d).transpose(0, 2, 1, 3).reshape(-1, _ROW, 8, _HW)


def _forward(A_x, A_c_kv, A_w_q, A_w_uk, A_w_uv, A_w_o, B_w1, B_w2, *,
             lead=7, pre_bursts=(40, 62, 48, 48, 26, 62, 48, 48, 26, 84), spin_pre=1, spin_loop=2,
             qk_split=(3, 3, 3, 3, 2, 2), pv_split=(5, 5, 6)):
    B, SQ, M = A_x.shape
    _, SK, C = A_c_kv.shape
    _, H, D = A_w_q.shape
    F = B_w1.shape[1]
    assert B == 1 and SQ == 1 and H == 32 and 2 * D == _HW and M == 2 * _HW and C == 2 * _HW
    assert F % 8 == 0 and 0 < lead < _RUN
    dt = A_x.dtype
    rows = (SK + 4 * H * D) // 4 // _ROW + 2 * -(-(F // 4) // _ROW)
    kernel = functools.partial(
        _kernel, n_sems=64, H=H, D=D, M=M, C=C, lead=lead, pre_bursts=pre_bursts,
        spin_pre=spin_pre, spin_loop=spin_loop, qk_split=qk_split, pv_split=pv_split, eps=1e-5)
    any_spec = pl.BlockSpec(memory_space=pl.ANY)
    out = pl.pallas_call(
        kernel,
        in_specs=[any_spec] * 8,
        out_specs=pl.BlockSpec(memory_space=pltpu.VMEM),
        out_shape=jax.ShapeDtypeStruct((1, M), dt),
        scratch_shapes=[
            pltpu.VMEM((1, M), dt),
            pltpu.VMEM((rows, _ROW, 8, _HW), dt),
            pltpu.VMEM((128, 128 * 8), _BF16),
            pltpu.SMEM((1,), jnp.int32),
        ],
        compiler_params=pltpu.CompilerParams(vmem_limit_bytes=100 * 1024 * 1024),
    )(
        A_x.reshape(1, M),
        _units(A_c_kv.reshape(SK, C)).reshape(-1, _ROW, 8, _HW),
        _head_units(A_w_q),
        _head_units(A_w_uk),
        _head_units(A_w_uv),
        _units(A_w_o.reshape(H * D, M)).reshape(-1, _ROW, 8, _HW),
        _units(B_w1.T),
        _units(B_w2),
    )
    return out.reshape(B, SQ, M)


@jax.jit
def pallas_recurrent_scan__compressed_kv_cla__dense_activation_silu__decode_kernel(
    A_x: jax.Array,
    A_c_kv: jax.Array,
    A_w_q: jax.Array,
    A_w_uk: jax.Array,
    A_w_uv: jax.Array,
    A_w_o: jax.Array,
    B_x: jax.Array,
    B_w1: jax.Array,
    B_w2: jax.Array,
):
    return _forward(A_x, A_c_kv, A_w_q, A_w_uk, A_w_uv, A_w_o, B_w1, B_w2)
```
